```python
import jax
import jax.numpy as jnp

def _softmax(x, axis=-1):
    return jax.nn.softmax(x, axis=axis)

def _gelu(x):
    return jax.nn.gelu(x, approximate=True)

def _silu(x):
    return jax.nn.silu(x)

def _sigmoid(x):
    return jax.nn.sigmoid(x)

def _layernorm(x, axis=-1, eps=1e-05):
    m = jnp.mean(x, axis=axis, keepdims=True)
    v = jnp.var(x, axis=axis, keepdims=True)
    return (x - m) / jnp.sqrt(v + eps)

def _scatter_add(tgt, idx, src, axis=0):
    return tgt.at[idx].add(src)

def _segment_sum(src, seg, n):
    return jax.ops.segment_sum(src, seg, n)

class _Rng:

    def __init__(self, key):
        self._k = key

    def _next(self):
        self._k, sub = jax.random.split(self._k)
        return sub

    def normal(self, shape):
        return jax.random.normal(self._next(), shape, dtype=jnp.bfloat16)

    def randint(self, lo, hi, shape):
        return jax.random.randint(self._next(), shape, lo, hi, dtype=jnp.int32)

    def uniform(self, shape, lo=0.0, hi=1.0):
        return jax.random.uniform(self._next(), shape, jnp.bfloat16, lo, hi)

    def permutation(self, n):
        return jax.random.permutation(self._next(), n)
kernel_name = 'interleave_layers__memory_aug_recurrent_mem_tr__glu_gated_swiglu__prompt'

def setup_inputs():
    _rng = _Rng(jax.random.key(int.from_bytes(__import__("os").urandom(4), "little")))
    _w = lambda a: (lambda t: t.astype(jnp.bfloat16) if jnp.issubdtype(t.dtype, jnp.floating) else t)(jnp.asarray(a))

    def _A_setup():
        B, S, Dm = (1, 2048, 576)
        H, Dh = (32, 128)
        M, seg = (8, 32)
        seg = min(seg, S)
        S = S // seg * seg
        return {'x': _w((lambda *s: _rng.normal(s) * 0.05)(B, S, Dm)), 'mem0': _w((lambda *s: _rng.normal(s) * 0.05)(B, M, Dm)), 'Wq': _w((lambda *s: _rng.normal(s) * 0.05)(Dm, H, Dh) * Dm ** (-0.5)), 'Wk': _w((lambda *s: _rng.normal(s) * 0.05)(Dm, H, Dh) * Dm ** (-0.5)), 'Wv': _w((lambda *s: _rng.normal(s) * 0.05)(Dm, H, Dh) * Dm ** (-0.5)), 'Wo': _w((lambda *s: _rng.normal(s) * 0.05)(H, Dh, Dm) * (H * Dh) ** (-0.5)), 'seg_len': seg}
    _A_in = _A_setup()

    def _B_setup():
        B, S, D, F = (1, 2048, 576, 4608)
        return {'x': _w((lambda *s: _rng.normal(s) * 0.05)(B, S, D)), 'w1': _w((lambda *s: _rng.normal(s) * 0.05)(D, F) * (2.0 / D) ** 0.5), 'w3': _w((lambda *s: _rng.normal(s) * 0.05)(D, F) * (2.0 / D) ** 0.5), 'w2': _w((lambda *s: _rng.normal(s) * 0.05)(F, D) * (2.0 / F) ** 0.5)}
    _B_in = _B_setup()
    return {'A_x': _A_in['x'], 'A_mem0': _A_in['mem0'], 'A_Wq': _A_in['Wq'], 'A_Wk': _A_in['Wk'], 'A_Wv': _A_in['Wv'], 'A_Wo': _A_in['Wo'], 'A_seg_len': _A_in['seg_len'], 'B_x': _B_in['x'], 'B_w1': _B_in['w1'], 'B_w3': _B_in['w3'], 'B_w2': _B_in['w2']}

def reference(A_x, A_mem0, A_Wq, A_Wk, A_Wv, A_Wo, A_seg_len, B_x, B_w1, B_w3, B_w2):

    def _A_ref(x, mem0, Wq, Wk, Wv, Wo, seg_len):
        B, S, Dm = x.shape
        H, Dh = (Wq.shape[1], Wq.shape[2])
        M = mem0.shape[1]
        scale = Dh ** (-0.5)
        n_seg = S // seg_len
        L = M + seg_len
        idx = jnp.arange(L)
        mask = (idx[:, None] < M) | (idx[:, None] >= idx[None, :])
        mem = mem0
        outs = []
        for s in range(n_seg):
            xs = x[:, s * seg_len:(s + 1) * seg_len, :].copy()
            h = jnp.concatenate([mem, xs], axis=1)
            q = jnp.einsum('btd,dhe->bhte', h, Wq)
            k = jnp.einsum('btd,dhe->bhte', h, Wk)
            v = jnp.einsum('btd,dhe->bhte', h, Wv)
            scores = jnp.einsum('bhqe,bhke->bhqk', q, k) * scale
            scores = jnp.where(mask[None, None], scores, -1000000000.0)
            p = _softmax(scores, axis=-1)
            o = jnp.einsum('bhqk,bhke->bhqe', p, v)
            o = jnp.einsum('bhte,hed->btd', o, Wo)
            mem = o[:, :M, :].copy()
            outs.append(o[:, M:, :])
        return jnp.concatenate(outs, axis=1)

    def _B_ref(x, w1, w3, w2):
        gate = jnp.einsum('bsd,df->bsf', x, w1)
        up = jnp.einsum('bsd,df->bsf', x, w3)
        h = _silu(gate) * up
        out = jnp.einsum('bsf,fd->bsd', h, w2)
        return out
    x = A_x
    x = x + _A_ref(_layernorm(x, axis=-1), A_mem0, A_Wq, A_Wk, A_Wv, A_Wo, A_seg_len)
    x = x + _B_ref(_layernorm(x, axis=-1), B_w1, B_w3, B_w2)
    x = x + _A_ref(_layernorm(x, axis=-1), A_mem0, A_Wq, A_Wk, A_Wv, A_Wo, A_seg_len)
    x = x + _B_ref(_layernorm(x, axis=-1), B_w1, B_w3, B_w2)
    return x
```

```python
import functools

import jax
import jax.numpy as jnp
from jax import lax
import jax.experimental.pallas as pl
import jax.experimental.pallas.tpu as pltpu

F32 = jnp.float32
BF16 = jnp.bfloat16
LAG = 3
HEAD_GROUP = 4
FF_CHUNK = 512
TOK_BLOCK = 128
NT_DIMS = (((1,), (1,)), ((), ()))


def _layernorm(x):
    mean = jnp.mean(x, axis=-1, keepdims=True)
    xc = x - mean
    var = jnp.mean(xc * xc, axis=-1, keepdims=True)
    return xc * lax.rsqrt(var + 1e-5)


def _kernel(xT_hbm, mem0_ref, wq_hbm, wk_hbm, wv_hbm, woT_hbm, w1_hbm, w3_hbm, w2T_hbm,
            outT_hbm,
            stage, wqkv, woT, w1, w3, w2T, xT, xs, outs,
            h_att, h_ffn, o_scr, act, res_new, res_old, res_x2, fill_scr, sems,
            *, seg, n_mem, n_heads, d_head):
    d_model, seq = xT.shape
    d_ff = w1.shape[1]
    n_seg = seq // seg
    m2 = 2 * n_mem
    rows = m2 + 2 * seg
    scale = d_head ** -0.5
    gw = 3 * d_head

    x_copy = pltpu.make_async_copy(xT_hbm, xT, sems.at[0])
    qkv_copies = [pltpu.make_async_copy(w, stage.at[i], sems.at[1 + i])
                  for i, w in enumerate((wq_hbm, wk_hbm, wv_hbm))]
    wo_copies = [pltpu.make_async_copy(woT_hbm.at[h], woT.at[:, pl.ds(h * d_head, d_head)], sems.at[4])
                 for h in range(n_heads)]
    w1_copy = pltpu.make_async_copy(w1_hbm, w1, sems.at[5])
    w3_copy = pltpu.make_async_copy(w3_hbm, w3, sems.at[6])
    w2_copy = pltpu.make_async_copy(w2T_hbm, w2T, sems.at[7])
    for c in [x_copy] + qkv_copies + wo_copies + [w1_copy, w3_copy, w2_copy]:
        c.start()

    ri = lax.broadcasted_iota(jnp.int32, (rows, rows), 0)
    ci = lax.broadcasted_iota(jnp.int32, (rows, rows), 1)

    def layer_of(i):
        return jnp.where(i < m2, i // n_mem, (i - m2) // seg)

    def pos_of(i):
        return jnp.where(i < m2, i % n_mem, n_mem + (i - m2) % seg)

    visible = (pos_of(ri) < n_mem) | (pos_of(ri) >= pos_of(ci))
    fill_scr[...] = jnp.where(layer_of(ri) == layer_of(ci),
                              jnp.where(visible, 0.0, -1e9), -jnp.inf).astype(F32)

    h_ffn[...] = jnp.zeros(h_ffn.shape, BF16)
    res_new[...] = jnp.zeros(res_new.shape, F32)
    res_old[...] = jnp.zeros(res_old.shape, F32)
    res_x2[...] = jnp.zeros(res_x2.shape, F32)

    x_copy.wait()
    for b in range(seq // TOK_BLOCK):
        blk = xT[:, b * TOK_BLOCK:(b + 1) * TOK_BLOCK].astype(F32)
        xs[b * TOK_BLOCK:(b + 1) * TOK_BLOCK, :] = blk.T.astype(BF16)

    mem0 = mem0_ref[...].astype(F32)
    h_att[0:m2, :] = jnp.concatenate([mem0, mem0], axis=0).astype(BF16)
    h_att[m2:m2 + seg, :] = _layernorm(xs[0:seg, :].astype(F32)).astype(BF16)
    h_att[m2 + seg:rows, :] = jnp.zeros((seg, d_model), BF16)

    for i in range(3):
        qkv_copies[i].wait()

        def regroup(blk, carry, i=i):
            src = pl.ds(pl.multiple_of(blk * (16 * n_heads), 16 * n_heads), 16 * n_heads)
            u = pltpu.bitcast(stage[i, src, :], jnp.uint32).reshape(8, 2, n_heads // 2, d_head)
            even = jnp.swapaxes(u[:, 0], 0, 1)
            odd = jnp.swapaxes(u[:, 1], 0, 1)
            lo = (even & jnp.uint32(0xFFFF)) | (odd << 16)
            hi = (even >> 16) | (odd & jnp.uint32(0xFFFF0000))
            dst = pl.ds(pl.multiple_of(blk * 16, 16), 16)
            for h in range(n_heads):
                col = (h % HEAD_GROUP) * gw + i * d_head
                word = (lo, hi)[h % 2][h // 2]
                wqkv[h // HEAD_GROUP, dst, col:col + d_head] = pltpu.bitcast(word, BF16)
            return carry

        lax.fori_loop(0, d_model // 16, regroup, 0)

    def seg_rows(s):
        return pl.ds(pl.multiple_of(s * seg, seg), seg)

    def attention():
        h = h_att[...]
        fill = fill_scr[...]
        keep = fill == 0.0
        for g in range(n_heads // HEAD_GROUP):
            qkv = jnp.dot(h, wqkv[g], preferred_element_type=F32).astype(BF16)
            for j in range(HEAD_GROUP):
                q = qkv[:, j * gw:j * gw + d_head]
                k = qkv[:, j * gw + d_head:j * gw + 2 * d_head]
                v = qkv[:, j * gw + 2 * d_head:(j + 1) * gw]
                s = lax.dot_general(q, k, NT_DIMS, preferred_element_type=F32)
                s = jnp.where(keep, s * scale, fill)
                e = jnp.exp(s - jnp.max(s, axis=-1, keepdims=True))
                inv = 1.0 / jnp.sum(e, axis=-1, keepdims=True)
                o = jnp.dot(e.astype(BF16), v, preferred_element_type=F32) * inv
                hd = g * HEAD_GROUP + j
                o_scr[:, hd * d_head:(hd + 1) * d_head] = o.astype(BF16)

    def ffn_down():
        return res_old[...] + lax.dot_general(act[...], w2T[...], NT_DIMS, preferred_element_type=F32)

    def out_proj():
        return lax.dot_general(o_scr[...], woT[...], NT_DIMS, preferred_element_type=F32)

    def ffn_up():
        h = h_ffn[...]
        for c in range(d_ff // FF_CHUNK):
            cols = slice(c * FF_CHUNK, (c + 1) * FF_CHUNK)
            gate = jnp.dot(h, w1[:, cols], preferred_element_type=F32)
            up = jnp.dot(h, w3[:, cols], preferred_element_type=F32)
            act[:, cols] = (gate * jax.nn.sigmoid(gate) * up).astype(BF16)

    def step(t, do_att, do_down, do_up, before_proj=None, before_up=None):
        if do_att:
            attention()
        if do_down:
            y = ffn_down()
            outs[seg_rows(jnp.clip(t - 2 - LAG, 0, n_seg - 1)), :] = y[seg:].astype(BF16)
        if do_att:
            if before_proj is not None:
                before_proj()
            a = out_proj()
            x1 = xs[seg_rows(jnp.minimum(t, n_seg - 1)), :].astype(F32) + a[m2:m2 + seg]
            x3 = res_x2[...] + a[m2 + seg:]
            mem_l2 = jnp.where(t < LAG, mem0_ref[...].astype(F32), a[n_mem:m2])
            h_att[0:m2, :] = jnp.concatenate([a[0:n_mem], mem_l2], axis=0).astype(BF16)
            nxt = xs[seg_rows(jnp.minimum(t + 1, n_seg - 1)), :].astype(F32)
            h_att[m2:m2 + seg, :] = _layernorm(nxt).astype(BF16)
        if do_down:
            res_x2[...] = y[:seg]
            h_att[m2 + seg:rows, :] = _layernorm(y[:seg]).astype(BF16)
        if do_up:
            if before_up is not None:
                before_up()
            ffn_up()
        res_old[...] = res_new[...]
        if do_att:
            res_new[0:seg, :] = x1
            res_new[seg:, :] = x3
            h_ffn[0:seg, :] = _layernorm(x1).astype(BF16)
            h_ffn[seg:, :] = _layernorm(x3).astype(BF16)

    def wait_wo():
        for c in wo_copies:
            c.wait()

    def wait_up():
        w1_copy.wait()
        w3_copy.wait()

    n_att = n_seg + LAG
    step(0, True, False, False, before_proj=wait_wo)
    step(1, True, False, True, before_up=wait_up)
    w2_copy.wait()

    def body(t, carry):
        step(t, True, True, True)
        return carry

    lax.fori_loop(2, n_att, body, 0)
    step(n_att, False, True, True)
    step(n_att + 1, False, True, False)

    for b in range(seq // TOK_BLOCK):
        blk = outs[b * TOK_BLOCK:(b + 1) * TOK_BLOCK, :].astype(F32)
        xT[:, b * TOK_BLOCK:(b + 1) * TOK_BLOCK] = blk.T.astype(BF16)
    out_copy = pltpu.make_async_copy(xT, outT_hbm, sems.at[0])
    out_copy.start()
    out_copy.wait()


@functools.partial(jax.jit, static_argnames=("A_seg_len",))
def pallas_interleave_layers__memory_aug_recurrent_mem_tr__glu_gated_swiglu__prompt_kernel(
    A_x: jax.Array,
    A_mem0: jax.Array,
    A_Wq: jax.Array,
    A_Wk: jax.Array,
    A_Wv: jax.Array,
    A_Wo: jax.Array,
    A_seg_len: int,
    B_x: jax.Array,
    B_w1: jax.Array,
    B_w3: jax.Array,
    B_w2: jax.Array,
):
    del B_x
    batch, seq, d_model = A_x.shape
    _, n_heads, d_head = A_Wq.shape
    n_mem = A_mem0.shape[1]
    d_ff = B_w1.shape[1]
    seg = int(A_seg_len)
    assert batch == 1 and seq % seg == 0 and seq % TOK_BLOCK == 0
    rows = 2 * (n_mem + seg)

    hbm = pl.BlockSpec(memory_space=pl.ANY)
    outT = pl.pallas_call(
        functools.partial(_kernel, seg=seg, n_mem=n_mem, n_heads=n_heads, d_head=d_head),
        out_shape=jax.ShapeDtypeStruct((d_model, seq), A_x.dtype),
        in_specs=[hbm, pl.BlockSpec(memory_space=pltpu.VMEM)] + [hbm] * 7,
        out_specs=hbm,
        scratch_shapes=[
            pltpu.VMEM((3, d_model * n_heads, d_head), BF16),
            pltpu.VMEM((n_heads // HEAD_GROUP, d_model, HEAD_GROUP * 3 * d_head), BF16),
            pltpu.VMEM((d_model, n_heads * d_head), BF16),
            pltpu.VMEM((d_model, d_ff), BF16),
            pltpu.VMEM((d_model, d_ff), BF16),
            pltpu.VMEM((d_model, d_ff), BF16),
            pltpu.VMEM((d_model, seq), BF16),
            pltpu.VMEM((seq, d_model), BF16),
            pltpu.VMEM((seq, d_model), BF16),
            pltpu.VMEM((rows, d_model), BF16),
            pltpu.VMEM((2 * seg, d_model), BF16),
            pltpu.VMEM((rows, n_heads * d_head), BF16),
            pltpu.VMEM((2 * seg, d_ff), BF16),
            pltpu.VMEM((2 * seg, d_model), F32),
            pltpu.VMEM((2 * seg, d_model), F32),
            pltpu.VMEM((seg, d_model), F32),
            pltpu.VMEM((rows, rows), F32),
            pltpu.SemaphoreType.DMA((8,)),
        ],
        compiler_params=pltpu.CompilerParams(vmem_limit_bytes=100 * 1024 * 1024),
    )(
        A_x[0].T,
        A_mem0[0],
        A_Wq.reshape(d_model * n_heads, d_head),
        A_Wk.reshape(d_model * n_heads, d_head),
        A_Wv.reshape(d_model * n_heads, d_head),
        jnp.transpose(A_Wo, (0, 2, 1)),
        B_w1,
        B_w3,
        B_w2.T,
    )
    return outT.T[None]
```

```python
import functools

import jax
import jax.numpy as jnp
from jax import lax
import jax.experimental.pallas as pl
import jax.experimental.pallas.tpu as pltpu

F32 = jnp.float32
BF16 = jnp.bfloat16
U32 = jnp.uint32
LANES = 128
LAG = 3
QK_DELAY = 1
PV_DELAY = 2
WO_CHUNKS = 4
TOK_BLOCK = 128
NT_DIMS = (((1,), (1,)), ((), ()))


def _layernorm(x):
    mean = jnp.mean(x, axis=-1, keepdims=True)
    xc = x - mean
    var = jnp.mean(xc * xc, axis=-1, keepdims=True)
    return xc * lax.rsqrt(var + 1e-5)


def _pack(x):
    return pltpu.bitcast(x.astype(BF16), U32)


def _load_slabs(ref, first, count, width=None):
    parts = [pltpu.bitcast(ref[first + i], BF16) for i in range(count)]
    if width is not None and width % LANES:
        parts[-1] = parts[-1][:, :width % LANES]
    return parts[0] if count == 1 else jnp.concatenate(parts, axis=1)


def _store_slabs(ref, row0, value):
    words = _pack(value)
    n_rows, width = words.shape
    for i in range(pl.cdiv(width, LANES)):
        part = words[:, i * LANES:min(width, (i + 1) * LANES)]
        ref[i, row0 // 2:row0 // 2 + n_rows, 0:part.shape[1]] = part


def _kernel(xT_hbm, mem0_ref, wq_hbm, wk_hbm, wv_hbm, woT_hbm, w1_hbm, w3_hbm, w2T_hbm,
            outT_hbm,
            qkv_stage, wo_stage, ff_stage, wqkv, woT, w1, w3, w2T, xT, xs, outs,
            h_att, h_ffn, o_scr, act, res_ffn, res_att, x2_buf, fill_scr, sems,
            *, seg, n_mem):
    d_model, seq = xT.shape
    n_heads, _, d_head = woT.shape
    n_ff = w1.shape[0]
    n_dm = h_att.shape[0]
    n_seg = seq // seg
    m2 = 2 * n_mem
    rows = m2 + 2 * seg
    scale = d_head ** -0.5

    x_copy = pltpu.make_async_copy(xT_hbm, xT, sems.at[0])
    qkv_copies = [pltpu.make_async_copy(w, qkv_stage.at[i], sems.at[1 + i])
                  for i, w in enumerate((wq_hbm, wk_hbm, wv_hbm))]
    wo_copy = pltpu.make_async_copy(woT_hbm, wo_stage, sems.at[4])
    ff_copies = [pltpu.make_async_copy(w, ff_stage.at[i], sems.at[5 + i])
                 for i, w in enumerate((w1_hbm, w3_hbm, w2T_hbm))]
    for c in [x_copy] + qkv_copies + [wo_copy] + ff_copies:
        c.start()

    ri = lax.broadcasted_iota(jnp.int32, (rows, rows), 0)
    ci = lax.broadcasted_iota(jnp.int32, (rows, rows), 1)

    def layer_of(i):
        return jnp.where(i < m2, i // n_mem, (i - m2) // seg)

    def pos_of(i):
        return jnp.where(i < m2, i % n_mem, n_mem + (i - m2) % seg)

    visible = (pos_of(ri) < n_mem) | (pos_of(ri) >= pos_of(ci))
    fill_scr[...] = jnp.where(layer_of(ri) == layer_of(ci),
                              jnp.where(visible, 0.0, -1e9), -jnp.inf).astype(F32)

    h_att[...] = jnp.zeros(h_att.shape, U32)
    h_ffn[...] = jnp.zeros(h_ffn.shape, U32)
    res_att[...] = jnp.zeros(res_att.shape, F32)
    x2_buf[...] = jnp.zeros(x2_buf.shape, F32)

    x_copy.wait()
    for b in range(seq // TOK_BLOCK):
        blk = xT[:, b * TOK_BLOCK:(b + 1) * TOK_BLOCK].astype(F32)
        xs[b * TOK_BLOCK:(b + 1) * TOK_BLOCK, :] = blk.T.astype(BF16)

    mem0 = mem0_ref[...].astype(F32)
    _store_slabs(h_att, 0, jnp.concatenate([mem0, mem0], axis=0))
    _store_slabs(h_att, m2, _layernorm(xs[0:seg, :].astype(F32)))

    for i in range(3):
        qkv_copies[i].wait()

        def regroup(blk, carry, i=i):
            src = pl.ds(pl.multiple_of(blk * (16 * n_heads), 16 * n_heads), 16 * n_heads)
            u = pltpu.bitcast(qkv_stage[i, src, :], U32).reshape(8, 2, n_heads // 2, d_head)
            even = jnp.swapaxes(u[:, 0], 0, 1)
            odd = jnp.swapaxes(u[:, 1], 0, 1)
            lo = (even & jnp.uint32(0xFFFF)) | (odd << 16)
            hi = (even >> 16) | (odd & jnp.uint32(0xFFFF0000))
            dst = pl.ds(pl.multiple_of(blk * 8, 8), 8)
            for h in range(n_heads):
                wqkv[3 * h + i, dst, :] = (lo, hi)[h % 2][h // 2]
            return carry

        lax.fori_loop(0, d_model // 16, regroup, 0)

    def prepare_wo():
        wo_copy.wait()

        def repack(h, carry):
            woT[h] = pltpu.bitcast(wo_stage[h], U32)
            return carry

        lax.fori_loop(0, n_heads, repack, 0)

    def prepare_ffn():
        for i, dst in enumerate((w1, w3, w2T)):
            ff_copies[i].wait()

            def repack(blk, carry, i=i, dst=dst):
                src = pl.ds(pl.multiple_of(blk * 16, 16), 16)
                words = pltpu.bitcast(ff_stage[i, src, :], U32)
                for c in range(n_ff):
                    dst[c, pl.ds(pl.multiple_of(blk * 8, 8), 8), :] = words[:, c * LANES:(c + 1) * LANES]
                return carry

            lax.fori_loop(0, d_model // 16, repack, 0)

    def seg_rows(s):
        return pl.ds(pl.multiple_of(s * seg, seg), seg)

    def project(hd):
        h = _load_slabs(h_att, 0, n_dm, d_model)
        qkv = jnp.dot(h, _load_slabs(wqkv, 3 * hd, 3), preferred_element_type=F32).astype(BF16)
        return tuple(qkv[:, i * d_head:(i + 1) * d_head] for i in range(3))

    def scores(q, k):
        s = lax.dot_general(q, k, NT_DIMS, preferred_element_type=F32)
        fill = fill_scr[...]
        s = jnp.where(fill == 0.0, s * scale, fill)
        e = jnp.exp(s - jnp.max(s, axis=-1, keepdims=True))
        total = jnp.sum(e, axis=-1, keepdims=True)
        inv = pl.reciprocal(total, approx=True)
        inv = inv * (2.0 - total * inv)
        return (e * inv).astype(BF16)

    def ffn_up(c):
        h = _load_slabs(h_ffn, 0, n_dm, d_model)
        w = jnp.concatenate([_load_slabs(w1, c, 1), _load_slabs(w3, c, 1)], axis=1)
        gate_up = jnp.dot(h, w, preferred_element_type=F32)
        half = 0.5 * gate_up[:, :LANES]
        act[c] = _pack((half * jnp.tanh(half) + half) * gate_up[:, LANES:])

    def contract(lhs, rhs, first, count):
        return lax.dot_general(_load_slabs(lhs, first, count), _load_slabs(rhs, first, count),
                               NT_DIMS, preferred_element_type=F32)

    def step(t, do_att, do_ffn, before_proj=None):
        qkv, probs = {}, {}

        def attention_slot(i):
            if 0 <= i - QK_DELAY < n_heads:
                q, k, _ = qkv[i - QK_DELAY]
                probs[i - QK_DELAY] = scores(q, k)
            if 0 <= i - PV_DELAY < n_heads:
                hd = i - PV_DELAY
                o_scr[hd] = _pack(jnp.dot(probs.pop(hd), qkv.pop(hd)[2], preferred_element_type=F32))

        ff_done = 0
        for i in range(n_heads):
            if do_att:
                qkv[i] = project(i)
            if do_ffn:
                while ff_done < (i + 1) * n_ff // n_heads:
                    ffn_up(ff_done)
                    ff_done += 1
            if do_att:
                attention_slot(i)

        if do_att:
            if before_proj is not None:
                before_proj()
            per = n_heads // WO_CHUNKS
            a = None
            for c in range(WO_CHUNKS):
                if c < PV_DELAY:
                    attention_slot(n_heads + c)
                part = contract(o_scr, woT, c * per, per)
                a = part if a is None else a + part
            x1 = xs[seg_rows(jnp.minimum(t, n_seg - 1)), :].astype(F32) + a[m2:m2 + seg]
            x3 = res_att[...] + a[m2 + seg:]
            mem_l2 = jnp.where(t < LAG, mem0_ref[...].astype(F32), a[n_mem:m2])
            _store_slabs(h_att, 0, jnp.concatenate([a[0:n_mem], mem_l2], axis=0))
            nxt = xs[seg_rows(jnp.minimum(t + 1, n_seg - 1)), :].astype(F32)
            _store_slabs(h_att, m2, _layernorm(nxt))
            x2 = x2_buf[...]
            res_att[...] = x2
            _store_slabs(h_att, m2 + seg, _layernorm(x2))
            _store_slabs(h_ffn, 0, _layernorm(x1))
            _store_slabs(h_ffn, seg, _layernorm(x3))
        if do_ffn:
            y = res_ffn[...] + contract(act, w2T, 0, n_ff)
            x2_buf[...] = y[:seg]
            outs[seg_rows(jnp.clip(t - 1 - LAG, 0, n_seg - 1)), :] = y[seg:].astype(BF16)
        if do_att:
            res_ffn[0:seg, :] = x1
            res_ffn[seg:, :] = x3

    n_att = n_seg + LAG
    step(0, True, False, before_proj=prepare_wo)
    prepare_ffn()

    def body(t, carry):
        step(t, True, True)
        return carry

    lax.fori_loop(1, n_att, body, 0)
    step(n_att, False, True)

    for b in range(seq // TOK_BLOCK):
        blk = outs[b * TOK_BLOCK:(b + 1) * TOK_BLOCK, :].astype(F32)
        xT[:, b * TOK_BLOCK:(b + 1) * TOK_BLOCK] = blk.T.astype(BF16)
    out_copy = pltpu.make_async_copy(xT, outT_hbm, sems.at[0])
    out_copy.start()
    out_copy.wait()


@functools.partial(jax.jit, static_argnames=("A_seg_len",))
def pallas_interleave_layers__memory_aug_recurrent_mem_tr__glu_gated_swiglu__prompt_kernel(
    A_x: jax.Array,
    A_mem0: jax.Array,
    A_Wq: jax.Array,
    A_Wk: jax.Array,
    A_Wv: jax.Array,
    A_Wo: jax.Array,
    A_seg_len: int,
    B_x: jax.Array,
    B_w1: jax.Array,
    B_w3: jax.Array,
    B_w2: jax.Array,
):
    del B_x
    batch, seq, d_model = A_x.shape
    _, n_heads, d_head = A_Wq.shape
    n_mem = A_mem0.shape[1]
    d_ff = B_w1.shape[1]
    seg = int(A_seg_len)
    assert batch == 1 and seq % seg == 0 and seq % TOK_BLOCK == 0
    assert d_head == LANES and d_ff % LANES == 0
    rows = 2 * (n_mem + seg)
    n_ff = d_ff // LANES
    n_dm = pl.cdiv(d_model, LANES)

    hbm = pl.BlockSpec(memory_space=pl.ANY)
    outT = pl.pallas_call(
        functools.partial(_kernel, seg=seg, n_mem=n_mem),
        out_shape=jax.ShapeDtypeStruct((d_model, seq), A_x.dtype),
        in_specs=[hbm, pl.BlockSpec(memory_space=pltpu.VMEM)] + [hbm] * 7,
        out_specs=hbm,
        scratch_shapes=[
            pltpu.VMEM((3, d_model * n_heads, d_head), BF16),
            pltpu.VMEM((n_heads, d_model, d_head), BF16),
            pltpu.VMEM((3, d_model, d_ff), BF16),
            pltpu.VMEM((3 * n_heads, d_model // 2, d_head), U32),
            pltpu.VMEM((n_heads, d_model // 2, d_head), U32),
            pltpu.VMEM((n_ff, d_model // 2, LANES), U32),
            pltpu.VMEM((n_ff, d_model // 2, LANES), U32),
            pltpu.VMEM((n_ff, d_model // 2, LANES), U32),
            pltpu.VMEM((d_model, seq), BF16),
            pltpu.VMEM((seq, d_model), BF16),
            pltpu.VMEM((seq, d_model), BF16),
            pltpu.VMEM((n_dm, rows // 2, LANES), U32),
            pltpu.VMEM((n_dm, seg, LANES), U32),
            pltpu.VMEM((n_heads, rows // 2, d_head), U32),
            pltpu.VMEM((n_ff, seg, LANES), U32),
            pltpu.VMEM((2 * seg, d_model), F32),
            pltpu.VMEM((seg, d_model), F32),
            pltpu.VMEM((seg, d_model), F32),
            pltpu.VMEM((rows, rows), F32),
            pltpu.SemaphoreType.DMA((8,)),
        ],
        compiler_params=pltpu.CompilerParams(vmem_limit_bytes=100 * 1024 * 1024),
    )(
        A_x[0].T,
        A_mem0[0],
        A_Wq.reshape(d_model * n_heads, d_head),
        A_Wk.reshape(d_model * n_heads, d_head),
        A_Wv.reshape(d_model * n_heads, d_head),
        jnp.transpose(A_Wo, (0, 2, 1)),
        B_w1,
        B_w3,
        B_w2.T,
    )
    return outT.T[None]
```

```python
import functools

import jax
import jax.numpy as jnp
from jax import lax
import jax.experimental.pallas as pl
import jax.experimental.pallas.tpu as pltpu

F32 = jnp.float32
BF16 = jnp.bfloat16
U32 = jnp.uint32
LANES = 128
LAG = 3
DELAYS_WITH_FFN = (1, 2)
DELAYS_ALONE = (2, 5)
WO_CHUNKS = 8
IN_FLIGHT = 2
TOK_BLOCK = 128
NT_DIMS = (((1,), (1,)), ((), ()))


def _layernorm(x):
    mean = jnp.mean(x, axis=-1, keepdims=True)
    xc = x - mean
    var = jnp.mean(xc * xc, axis=-1, keepdims=True)
    return xc * lax.rsqrt(var + 1e-5)


def _pack(x):
    return pltpu.bitcast(x.astype(BF16), U32)


def _load_slabs(ref, first, count, n_rows=None, width=None):
    words = ref.shape[1] if n_rows is None else n_rows // 2
    lanes = [LANES] * count
    if width is not None and width % LANES:
        lanes[-1] = width % LANES
    parts = [pltpu.bitcast(ref[first + i, 0:words, 0:lanes[i]], BF16) for i in range(count)]
    return parts[0] if count == 1 else jnp.concatenate(parts, axis=1)


def _store_slabs(ref, row0, value):
    words = _pack(value)
    n_rows, width = words.shape
    for i in range(pl.cdiv(width, LANES)):
        part = words[:, i * LANES:min(width, (i + 1) * LANES)]
        ref[i, row0 // 2:row0 // 2 + n_rows, 0:part.shape[1]] = part


def _kernel(xT_hbm, mem0_ref, wq_hbm, wk_hbm, wv_hbm, woT_hbm, w1_hbm, w3_hbm, w2T_hbm,
            outT_hbm,
            qkv_stage, wqkv, woT, w1, w3, w2T, xT, xs, outs,
            h_att, h_ffn, o_scr, act, res_ffn, res_att, x2_buf, fill_scr, sems,
            *, seg, n_mem):
    d_model, seq = xT.shape
    n_heads, _, d_head = woT.shape
    n_ff = w1.shape[0]
    n_dm = h_att.shape[0]
    n_seg = seq // seg
    m2 = 2 * n_mem
    rows = m2 + 2 * seg
    scale = d_head ** -0.5

    n_blk = seq // TOK_BLOCK

    def block(b):
        return slice(b * TOK_BLOCK, (b + 1) * TOK_BLOCK)

    def slab_copies(src, dst, sem):
        words = src.bitcast(U32)
        return [pltpu.make_async_copy(words.at[:, pl.ds(c * LANES, LANES)], dst.at[c], sem)
                for c in range(n_ff)]

    head, tail = pl.ds(0, TOK_BLOCK), pl.ds(TOK_BLOCK, seq - TOK_BLOCK)
    loads = [
        [pltpu.make_async_copy(xT_hbm.at[:, head], xT.at[:, head], sems.at[0])],
        [pltpu.make_async_copy(wq_hbm, qkv_stage.at[0], sems.at[1])],
        [pltpu.make_async_copy(wk_hbm, qkv_stage.at[1], sems.at[2])],
        [pltpu.make_async_copy(wv_hbm, qkv_stage.at[2], sems.at[3])],
        [pltpu.make_async_copy(woT_hbm.bitcast(U32), woT, sems.at[4])],
        slab_copies(w1_hbm, w1, sems.at[5]),
        slab_copies(w3_hbm, w3, sems.at[6]),
        slab_copies(w2T_hbm, w2T, sems.at[7]),
        [pltpu.make_async_copy(xT_hbm.at[:, tail], xT.at[:, tail], sems.at[8])],
    ]

    def start_load(i):
        if i < len(loads):
            for c in loads[i]:
                c.start()

    def finish_load(i):
        for c in loads[i]:
            c.wait()
        start_load(i + IN_FLIGHT)

    for i in range(IN_FLIGHT):
        start_load(i)

    ri = lax.broadcasted_iota(jnp.int32, (rows, rows), 0)
    ci = lax.broadcasted_iota(jnp.int32, (rows, rows), 1)

    def layer_of(i):
        return jnp.where(i < m2, i // n_mem, (i - m2) // seg)

    def pos_of(i):
        return jnp.where(i < m2, i % n_mem, n_mem + (i - m2) % seg)

    visible = (pos_of(ri) < n_mem) | (pos_of(ri) >= pos_of(ci))
    fill_scr[...] = jnp.where(layer_of(ri) == layer_of(ci),
                              jnp.where(visible, 0.0, -1e9), -jnp.inf).astype(F32)

    def transpose_in(b):
        xs[block(b), :] = xT[:, block(b)].astype(F32).T.astype(BF16)

    def transpose_out(b):
        xT[:, block(b)] = outs[block(b), :].astype(F32).T.astype(BF16)

    finish_load(0)
    transpose_in(0)
    mem0 = mem0_ref[...].astype(F32)
    _store_slabs(h_att, 0, jnp.concatenate([mem0, mem0], axis=0))
    _store_slabs(h_att, m2, _layernorm(xs[0:seg, :].astype(F32)))

    for i in range(3):
        finish_load(1 + i)

        def regroup(blk, carry, i=i):
            src = pl.ds(pl.multiple_of(blk * (16 * n_heads), 16 * n_heads), 16 * n_heads)
            u = pltpu.bitcast(qkv_stage[i, src, :], U32).reshape(8, 2, n_heads // 2, d_head)
            even = jnp.swapaxes(u[:, 0], 0, 1)
            odd = jnp.swapaxes(u[:, 1], 0, 1)
            lo = (even & jnp.uint32(0xFFFF)) | (odd << 16)
            hi = (even >> 16) | (odd & jnp.uint32(0xFFFF0000))
            dst = pl.ds(pl.multiple_of(blk * 8, 8), 8)
            for h in range(n_heads):
                wqkv[3 * h + i, dst, :] = (lo, hi)[h % 2][h // 2]
            return carry

        lax.fori_loop(0, d_model // 16, regroup, 0)

    def seg_rows(s):
        if isinstance(s, int):
            return pl.ds(s * seg, seg)
        return pl.ds(pl.multiple_of(s * seg, seg), seg)

    def x_seg(s):
        return xs[seg_rows(s), :].astype(F32)

    def project(hd, n):
        h = _load_slabs(h_att, 0, n_dm, n, d_model)
        qkv = jnp.dot(h, _load_slabs(wqkv, 3 * hd, 3), preferred_element_type=F32).astype(BF16)
        return tuple(qkv[:, i * d_head:(i + 1) * d_head] for i in range(3))

    def scores(q, k):
        n = q.shape[0]
        s = lax.dot_general(q, k, NT_DIMS, preferred_element_type=F32)
        fill = fill_scr[0:n, 0:n]
        s = jnp.where(fill == 0.0, s * scale, fill)
        e = jnp.exp(s - jnp.max(s, axis=-1, keepdims=True))
        total = jnp.sum(e, axis=-1, keepdims=True)
        inv = pl.reciprocal(total, approx=True)
        inv = inv * (2.0 - total * inv)
        return (e * inv).astype(BF16)

    def ffn_up(c, n):
        h = _load_slabs(h_ffn, 0, n_dm, n, d_model)
        w = jnp.concatenate([_load_slabs(w1, c, 1), _load_slabs(w3, c, 1)], axis=1)
        gate_up = jnp.dot(h, w, preferred_element_type=F32)
        half = 0.5 * gate_up[:, :LANES]
        act[c, 0:n // 2, :] = _pack((half * jnp.tanh(half) + half) * gate_up[:, LANES:])

    def contract(lhs, rhs, first, count, n):
        return lax.dot_general(_load_slabs(lhs, first, count, n), _load_slabs(rhs, first, count),
                               NT_DIMS, preferred_element_type=F32)

    def mix(n_att, n_ffn, before_proj=None, side_work=()):
        qk_delay, pv_delay = DELAYS_WITH_FFN if n_ffn else DELAYS_ALONE
        qkv, probs = {}, {}
        side_work = list(side_work)

        def attention_slot(i):
            if 0 <= i - qk_delay < n_heads:
                q, k, _ = qkv[i - qk_delay]
                probs[i - qk_delay] = scores(q, k)
            if 0 <= i - pv_delay < n_heads:
                hd = i - pv_delay
                o = jnp.dot(probs.pop(hd), qkv.pop(hd)[2], preferred_element_type=F32)
                o_scr[hd, 0:n_att // 2, :] = _pack(o)

        ff_done = 0
        for i in range(n_heads):
            qkv[i] = project(i, n_att)
            while n_ffn and ff_done < (i + 1) * n_ff // n_heads:
                ffn_up(ff_done, n_ffn)
                ff_done += 1
            attention_slot(i)
            if side_work:
                side_work.pop(0)()
        if before_proj is not None:
            before_proj()
        per = n_heads // WO_CHUNKS
        assert pv_delay < WO_CHUNKS and pv_delay <= n_heads - per
        a = None
        for c in range(WO_CHUNKS):
            part = contract(o_scr, woT, c * per, per, n_att)
            a = part if a is None else a + part
            if c < pv_delay:
                attention_slot(n_heads + c)
        return a

    def ffn_down(n):
        return res_ffn[0:n, :] + contract(act, w2T, 0, n_ff, n)

    def queue_ffn(slot, x):
        res_ffn[slot * seg:(slot + 1) * seg, :] = x
        _store_slabs(h_ffn, slot * seg, _layernorm(x))

    def set_memory(first, second):
        _store_slabs(h_att, 0, jnp.concatenate([first, second], axis=0))

    one = m2 + seg

    for t in range(LAG):
        last = t == LAG - 1
        if last:
            finish_load(5)
            finish_load(6)
        a = mix(one, 2 * seg if last else 0,
                before_proj=functools.partial(finish_load, 4) if t == 0 else None)
        set_memory(a[0:n_mem], mem0)
        _store_slabs(h_att, m2, _layernorm(x_seg(t + 1)))
        if last:
            finish_load(7)
            y = ffn_down(2 * seg)
            res_att[...] = y[:seg]
            _store_slabs(h_att, one, _layernorm(y[:seg]))
            x2_buf[...] = y[seg:]
        queue_ffn(t % 2, x_seg(t) + a[m2:])
    finish_load(8)
    for b in range(1, n_blk):
        transpose_in(b)

    def body(t, carry):
        a = mix(rows, 2 * seg)
        x1 = x_seg(t) + a[m2:one]
        x3 = res_att[...] + a[one:]
        set_memory(a[0:n_mem], a[n_mem:m2])
        _store_slabs(h_att, m2, _layernorm(x_seg(jnp.minimum(t + 1, n_seg - 1))))
        x2 = x2_buf[...]
        res_att[...] = x2
        _store_slabs(h_att, one, _layernorm(x2))
        y = ffn_down(2 * seg)
        x2_buf[...] = y[:seg]
        outs[seg_rows(jnp.maximum(t - 1 - LAG, 0)), :] = y[seg:].astype(BF16)
        queue_ffn(0, x1)
        queue_ffn(1, x3)
        return carry

    lax.fori_loop(LAG, n_seg, body, 0)

    done_blk = (n_seg - 1 - LAG) * seg // TOK_BLOCK
    early, late = pl.ds(0, done_blk * TOK_BLOCK), pl.ds(done_blk * TOK_BLOCK, seq - done_blk * TOK_BLOCK)
    out_early = pltpu.make_async_copy(xT.at[:, early], outT_hbm.at[:, early], sems.at[0])
    out_late = pltpu.make_async_copy(xT.at[:, late], outT_hbm.at[:, late], sems.at[1])

    mem = _load_slabs(h_att, 0, n_dm, m2, d_model).astype(F32)[n_mem:m2]
    x2 = res_att[...]
    for i in range(LAG):
        set_memory(mem, mem)
        _store_slabs(h_att, m2, _layernorm(x2))
        if i == 0:
            a = mix(one, 2 * seg)
            y = ffn_down(2 * seg)
            outs[seg_rows(n_seg - 1 - LAG), :] = y[seg:].astype(BF16)
            upcoming = [x2_buf[...], y[:seg]]
        elif i == 1:
            a = mix(one, 0, side_work=[functools.partial(transpose_out, b) for b in range(done_blk)])
            out_early.start()
        else:
            a = mix(one, 0)
        queue_ffn(i, x2 + a[m2:])
        mem = a[0:n_mem]
        if upcoming:
            x2 = upcoming.pop(0)
    for c in range(n_ff):
        ffn_up(c, LAG * seg)
    outs[(n_seg - LAG) * seg:, :] = ffn_down(LAG * seg).astype(BF16)
    for b in range(done_blk, n_blk):
        transpose_out(b)
    out_late.start()
    out_early.wait()
    out_late.wait()


@functools.partial(jax.jit, static_argnames=("A_seg_len",))
def pallas_interleave_layers__memory_aug_recurrent_mem_tr__glu_gated_swiglu__prompt_kernel(
    A_x: jax.Array,
    A_mem0: jax.Array,
    A_Wq: jax.Array,
    A_Wk: jax.Array,
    A_Wv: jax.Array,
    A_Wo: jax.Array,
    A_seg_len: int,
    B_x: jax.Array,
    B_w1: jax.Array,
    B_w3: jax.Array,
    B_w2: jax.Array,
):
    del B_x
    batch, seq, d_model = A_x.shape
    _, n_heads, d_head = A_Wq.shape
    n_mem = A_mem0.shape[1]
    d_ff = B_w1.shape[1]
    seg = int(A_seg_len)
    assert batch == 1 and seq % seg == 0 and seq % TOK_BLOCK == 0
    assert d_head == LANES and d_ff % LANES == 0
    rows = 2 * (n_mem + seg)
    n_ff = d_ff // LANES
    n_dm = pl.cdiv(d_model, LANES)

    hbm = pl.BlockSpec(memory_space=pl.ANY)
    outT = pl.pallas_call(
        functools.partial(_kernel, seg=seg, n_mem=n_mem),
        out_shape=jax.ShapeDtypeStruct((d_model, seq), A_x.dtype),
        in_specs=[hbm, pl.BlockSpec(memory_space=pltpu.VMEM)] + [hbm] * 7,
        out_specs=hbm,
        scratch_shapes=[
            pltpu.VMEM((3, d_model * n_heads, d_head), BF16),
            pltpu.VMEM((3 * n_heads, d_model // 2, d_head), U32),
            pltpu.VMEM((n_heads, d_model // 2, d_head), U32),
            pltpu.VMEM((n_ff, d_model // 2, LANES), U32),
            pltpu.VMEM((n_ff, d_model // 2, LANES), U32),
            pltpu.VMEM((n_ff, d_model // 2, LANES), U32),
            pltpu.VMEM((d_model, seq), BF16),
            pltpu.VMEM((seq, d_model), BF16),
            pltpu.VMEM((seq, d_model), BF16),
            pltpu.VMEM((n_dm, rows // 2, LANES), U32),
            pltpu.VMEM((n_dm, LAG * seg // 2, LANES), U32),
            pltpu.VMEM((n_heads, rows // 2, d_head), U32),
            pltpu.VMEM((n_ff, LAG * seg // 2, LANES), U32),
            pltpu.VMEM((LAG * seg, d_model), F32),
            pltpu.VMEM((seg, d_model), F32),
            pltpu.VMEM((seg, d_model), F32),
            pltpu.VMEM((rows, rows), F32),
            pltpu.SemaphoreType.DMA((9,)),
        ],
        compiler_params=pltpu.CompilerParams(vmem_limit_bytes=100 * 1024 * 1024),
    )(
        A_x[0].T,
        A_mem0[0],
        A_Wq.reshape(d_model * n_heads, d_head),
        A_Wk.reshape(d_model * n_heads, d_head),
        A_Wv.reshape(d_model * n_heads, d_head),
        jnp.transpose(A_Wo, (0, 2, 1)),
        B_w1,
        B_w3,
        B_w2.T,
    )
    return outT.T[None]
```

```python
import functools

import jax
import jax.numpy as jnp
from jax import lax
import jax.experimental.pallas as pl
import jax.experimental.pallas.tpu as pltpu

F32 = jnp.float32
BF16 = jnp.bfloat16
U32 = jnp.uint32
LANES = 128
LAG = 3
PLAN_WITH_FFN = (1, 2, 8, 2)
PLAN_ALONE = (2, 5, 16, 2)
IN_FLIGHT = 2
TOK_BLOCK = 128
NT_DIMS = (((1,), (1,)), ((), ()))


def _layernorm(x):
    mean = jnp.mean(x, axis=-1, keepdims=True)
    xc = x - mean
    var = jnp.mean(xc * xc, axis=-1, keepdims=True)
    return xc * lax.rsqrt(var + 1e-5)


def _pack(x):
    return pltpu.bitcast(x.astype(BF16), U32)


def _load_slabs(ref, first, count, n_rows=None, width=None):
    words = ref.shape[1] if n_rows is None else n_rows // 2
    lanes = [LANES] * count
    if width is not None and width % LANES:
        lanes[-1] = width % LANES
    parts = [pltpu.bitcast(ref[first + i, 0:words, 0:lanes[i]], BF16) for i in range(count)]
    return parts[0] if count == 1 else jnp.concatenate(parts, axis=1)


def _store_slabs(ref, row0, value):
    words = _pack(value)
    n_rows, width = words.shape
    for i in range(pl.cdiv(width, LANES)):
        part = words[:, i * LANES:min(width, (i + 1) * LANES)]
        ref[i, row0 // 2:row0 // 2 + n_rows, 0:part.shape[1]] = part


def _kernel(xT_hbm, mem0_ref, wq_hbm, wk_hbm, wv_hbm, woT_hbm, w1_hbm, w3_hbm, w2T_hbm,
            outT_hbm,
            qkv_stage, wqkv, woT, w1, w3, w2T, xT, xs, outs,
            h_att, h_ffn, o_scr, act, res_ffn, res_att, x2_buf, fill_scr, sems,
            *, seg, n_mem):
    d_model, seq = xT.shape
    n_heads, _, d_head = woT.shape
    n_ff = w1.shape[0]
    n_dm = h_att.shape[0]
    n_seg = seq // seg
    m2 = 2 * n_mem
    rows = m2 + 2 * seg
    scale = d_head ** -0.5

    n_blk = seq // TOK_BLOCK

    def block(b):
        return slice(b * TOK_BLOCK, (b + 1) * TOK_BLOCK)

    def slab_copies(src, dst, sem):
        words = src.bitcast(U32)
        return [pltpu.make_async_copy(words.at[:, pl.ds(c * LANES, LANES)], dst.at[c], sem)
                for c in range(n_ff)]

    head, tail = pl.ds(0, TOK_BLOCK), pl.ds(TOK_BLOCK, seq - TOK_BLOCK)
    loads = [
        [pltpu.make_async_copy(xT_hbm.at[:, head], xT.at[:, head], sems.at[0])],
        [pltpu.make_async_copy(wq_hbm, qkv_stage.at[0], sems.at[1])],
        [pltpu.make_async_copy(wk_hbm, qkv_stage.at[1], sems.at[2])],
        [pltpu.make_async_copy(wv_hbm, qkv_stage.at[2], sems.at[3])],
        [pltpu.make_async_copy(woT_hbm.bitcast(U32), woT, sems.at[4])],
        slab_copies(w1_hbm, w1, sems.at[5]),
        slab_copies(w3_hbm, w3, sems.at[6]),
        slab_copies(w2T_hbm, w2T, sems.at[7]),
        [pltpu.make_async_copy(xT_hbm.at[:, tail], xT.at[:, tail], sems.at[8])],
    ]

    def start_load(i):
        if i < len(loads):
            for c in loads[i]:
                c.start()

    def finish_load(i):
        for c in loads[i]:
            c.wait()
        start_load(i + IN_FLIGHT)

    for i in range(IN_FLIGHT):
        start_load(i)

    ri = lax.broadcasted_iota(jnp.int32, (rows, rows), 0)
    ci = lax.broadcasted_iota(jnp.int32, (rows, rows), 1)

    def layer_of(i):
        return jnp.where(i < m2, i // n_mem, (i - m2) // seg)

    def pos_of(i):
        return jnp.where(i < m2, i % n_mem, n_mem + (i - m2) % seg)

    visible = (pos_of(ri) < n_mem) | (pos_of(ri) >= pos_of(ci))
    fill_scr[...] = jnp.where(layer_of(ri) == layer_of(ci),
                              jnp.where(visible, 0.0, -1e9), -jnp.inf).astype(F32)

    def transpose_in(b):
        xs[block(b), :] = xT[:, block(b)].astype(F32).T.astype(BF16)

    def transpose_out(b):
        xT[:, block(b)] = outs[block(b), :].astype(F32).T.astype(BF16)

    finish_load(0)
    transpose_in(0)
    mem0 = mem0_ref[...].astype(F32)
    _store_slabs(h_att, 0, jnp.concatenate([mem0, mem0], axis=0))
    _store_slabs(h_att, m2, _layernorm(xs[0:seg, :].astype(F32)))

    for i in range(3):
        finish_load(1 + i)

        def regroup(blk, carry, i=i):
            src = pl.ds(pl.multiple_of(blk * (16 * n_heads), 16 * n_heads), 16 * n_heads)
            u = pltpu.bitcast(qkv_stage[i, src, :], U32).reshape(8, 2, n_heads // 2, d_head)
            even = jnp.swapaxes(u[:, 0], 0, 1)
            odd = jnp.swapaxes(u[:, 1], 0, 1)
            lo = (even & jnp.uint32(0xFFFF)) | (odd << 16)
            hi = (even >> 16) | (odd & jnp.uint32(0xFFFF0000))
            dst = pl.ds(pl.multiple_of(blk * 8, 8), 8)
            for h in range(n_heads):
                wqkv[3 * h + i, dst, :] = (lo, hi)[h % 2][h // 2]
            return carry

        lax.fori_loop(0, d_model // 16, regroup, 0)

    def seg_rows(s):
        if isinstance(s, int):
            return pl.ds(s * seg, seg)
        return pl.ds(pl.multiple_of(s * seg, seg), seg)

    def x_seg(s):
        return xs[seg_rows(s), :].astype(F32)

    def project(hd, n):
        h = _load_slabs(h_att, 0, n_dm, n, d_model)
        qkv = jnp.dot(h, _load_slabs(wqkv, 3 * hd, 3), preferred_element_type=F32).astype(BF16)
        return tuple(qkv[:, i * d_head:(i + 1) * d_head] for i in range(3))

    def scores(q, k):
        n = q.shape[0]
        s = lax.dot_general(q, k, NT_DIMS, preferred_element_type=F32)
        fill = fill_scr[0:n, 0:n]
        s = jnp.where(fill == 0.0, s * scale, fill)
        e = jnp.exp(s - jnp.max(s, axis=-1, keepdims=True))
        total = jnp.sum(e, axis=-1, keepdims=True)
        inv = pl.reciprocal(total, approx=True)
        inv = inv * (2.0 - total * inv)
        return (e * inv).astype(BF16)

    def ffn_up(c, n):
        h = _load_slabs(h_ffn, 0, n_dm, n, d_model)
        w = jnp.concatenate([_load_slabs(w1, c, 1), _load_slabs(w3, c, 1)], axis=1)
        gate_up = jnp.dot(h, w, preferred_element_type=F32)
        half = 0.5 * gate_up[:, :LANES]
        act[c, 0:n // 2, :] = _pack((half * jnp.tanh(half) + half) * gate_up[:, LANES:])

    def contract(lhs, rhs, first, count, n):
        return lax.dot_general(_load_slabs(lhs, first, count, n), _load_slabs(rhs, first, count),
                               NT_DIMS, preferred_element_type=F32)

    def mix(n_att, n_ffn, before_proj=None, side_work=()):
        qk_delay, pv_delay, n_chunks, spacing = PLAN_WITH_FFN if n_ffn else PLAN_ALONE
        qkv, probs = {}, {}
        side_work = list(side_work)

        def attention_slot(i):
            if 0 <= i - qk_delay < n_heads:
                q, k, _ = qkv[i - qk_delay]
                probs[i - qk_delay] = scores(q, k)
            if 0 <= i - pv_delay < n_heads:
                hd = i - pv_delay
                o = jnp.dot(probs.pop(hd), qkv.pop(hd)[2], preferred_element_type=F32)
                o_scr[hd, 0:n_att // 2, :] = _pack(o)

        ff_done = 0
        for i in range(n_heads):
            qkv[i] = project(i, n_att)
            while n_ffn and ff_done < (i + 1) * n_ff // n_heads:
                ffn_up(ff_done, n_ffn)
                ff_done += 1
            attention_slot(i)
            if side_work:
                side_work.pop(0)()
        if before_proj is not None:
            before_proj()
        per = n_heads // n_chunks
        assert pv_delay * spacing * per <= n_heads - pv_delay
        a = None
        for c in range(n_chunks):
            part = contract(o_scr, woT, c * per, per, n_att)
            a = part if a is None else a + part
            if (c + 1) % spacing == 0:
                attention_slot(n_heads + c // spacing)
        return a

    def ffn_down(n):
        return res_ffn[0:n, :] + contract(act, w2T, 0, n_ff, n)

    def queue_ffn(slot, x):
        res_ffn[slot * seg:(slot + 1) * seg, :] = x
        _store_slabs(h_ffn, slot * seg, _layernorm(x))

    def set_memory(first, second):
        _store_slabs(h_att, 0, jnp.concatenate([first, second], axis=0))

    one = m2 + seg

    for t in range(LAG):
        last = t == LAG - 1
        if last:
            finish_load(5)
            finish_load(6)
        a = mix(one, 2 * seg if last else 0,
                before_proj=functools.partial(finish_load, 4) if t == 0 else None)
        set_memory(a[0:n_mem], mem0)
        _store_slabs(h_att, m2, _layernorm(x_seg(t + 1)))
        if last:
            finish_load(7)
            y = ffn_down(2 * seg)
            res_att[...] = y[:seg]
            _store_slabs(h_att, one, _layernorm(y[:seg]))
            x2_buf[...] = y[seg:]
        queue_ffn(t % 2, x_seg(t) + a[m2:])
    finish_load(8)
    for b in range(1, n_blk):
        transpose_in(b)

    def body(t, carry):
        a = mix(rows, 2 * seg)
        x1 = x_seg(t) + a[m2:one]
        x3 = res_att[...] + a[one:]
        set_memory(a[0:n_mem], a[n_mem:m2])
        _store_slabs(h_att, m2, _layernorm(x_seg(jnp.minimum(t + 1, n_seg - 1))))
        x2 = x2_buf[...]
        res_att[...] = x2
        _store_slabs(h_att, one, _layernorm(x2))
        y = ffn_down(2 * seg)
        x2_buf[...] = y[:seg]
        outs[seg_rows(jnp.maximum(t - 1 - LAG, 0)), :] = y[seg:].astype(BF16)
        queue_ffn(0, x1)
        queue_ffn(1, x3)
        return carry

    lax.fori_loop(LAG, n_seg, body, 0)

    done_blk = (n_seg - 1 - LAG) * seg // TOK_BLOCK
    early, late = pl.ds(0, done_blk * TOK_BLOCK), pl.ds(done_blk * TOK_BLOCK, seq - done_blk * TOK_BLOCK)
    out_early = pltpu.make_async_copy(xT.at[:, early], outT_hbm.at[:, early], sems.at[0])
    out_late = pltpu.make_async_copy(xT.at[:, late], outT_hbm.at[:, late], sems.at[1])

    mem = _load_slabs(h_att, 0, n_dm, m2, d_model).astype(F32)[n_mem:m2]
    x2 = res_att[...]
    for i in range(LAG):
        set_memory(mem, mem)
        _store_slabs(h_att, m2, _layernorm(x2))
        if i == 0:
            a = mix(one, 2 * seg)
            y = ffn_down(2 * seg)
            outs[seg_rows(n_seg - 1 - LAG), :] = y[seg:].astype(BF16)
            upcoming = [x2_buf[...], y[:seg]]
        elif i == 1:
            a = mix(one, 0, side_work=[functools.partial(transpose_out, b) for b in range(done_blk)])
            out_early.start()
        else:
            a = mix(one, 0)
        queue_ffn(i, x2 + a[m2:])
        mem = a[0:n_mem]
        if upcoming:
            x2 = upcoming.pop(0)
    for c in range(n_ff):
        ffn_up(c, LAG * seg)
    outs[(n_seg - LAG) * seg:, :] = ffn_down(LAG * seg).astype(BF16)
    for b in range(done_blk, n_blk):
        transpose_out(b)
    out_late.start()
    out_early.wait()
    out_late.wait()


@functools.partial(jax.jit, static_argnames=("A_seg_len",))
def pallas_interleave_layers__memory_aug_recurrent_mem_tr__glu_gated_swiglu__prompt_kernel(
    A_x: jax.Array,
    A_mem0: jax.Array,
    A_Wq: jax.Array,
    A_Wk: jax.Array,
    A_Wv: jax.Array,
    A_Wo: jax.Array,
    A_seg_len: int,
    B_x: jax.Array,
    B_w1: jax.Array,
    B_w3: jax.Array,
    B_w2: jax.Array,
):
    del B_x
    batch, seq, d_model = A_x.shape
    _, n_heads, d_head = A_Wq.shape
    n_mem = A_mem0.shape[1]
    d_ff = B_w1.shape[1]
    seg = int(A_seg_len)
    assert batch == 1 and seq % seg == 0 and seq % TOK_BLOCK == 0
    assert d_head == LANES and d_ff % LANES == 0
    rows = 2 * (n_mem + seg)
    n_ff = d_ff // LANES
    n_dm = pl.cdiv(d_model, LANES)

    hbm = pl.BlockSpec(memory_space=pl.ANY)
    outT = pl.pallas_call(
        functools.partial(_kernel, seg=seg, n_mem=n_mem),
        out_shape=jax.ShapeDtypeStruct((d_model, seq), A_x.dtype),
        in_specs=[hbm, pl.BlockSpec(memory_space=pltpu.VMEM)] + [hbm] * 7,
        out_specs=hbm,
        scratch_shapes=[
            pltpu.VMEM((3, d_model * n_heads, d_head), BF16),
            pltpu.VMEM((3 * n_heads, d_model // 2, d_head), U32),
            pltpu.VMEM((n_heads, d_model // 2, d_head), U32),
            pltpu.VMEM((n_ff, d_model // 2, LANES), U32),
            pltpu.VMEM((n_ff, d_model // 2, LANES), U32),
            pltpu.VMEM((n_ff, d_model // 2, LANES), U32),
            pltpu.VMEM((d_model, seq), BF16),
            pltpu.VMEM((seq, d_model), BF16),
            pltpu.VMEM((seq, d_model), BF16),
            pltpu.VMEM((n_dm, rows // 2, LANES), U32),
            pltpu.VMEM((n_dm, LAG * seg // 2, LANES), U32),
            pltpu.VMEM((n_heads, rows // 2, d_head), U32),
            pltpu.VMEM((n_ff, LAG * seg // 2, LANES), U32),
            pltpu.VMEM((LAG * seg, d_model), F32),
            pltpu.VMEM((seg, d_model), F32),
            pltpu.VMEM((seg, d_model), F32),
            pltpu.VMEM((rows, rows), F32),
            pltpu.SemaphoreType.DMA((9,)),
        ],
        compiler_params=pltpu.CompilerParams(vmem_limit_bytes=100 * 1024 * 1024),
    )(
        A_x[0].T,
        A_mem0[0],
        A_Wq.reshape(d_model * n_heads, d_head),
        A_Wk.reshape(d_model * n_heads, d_head),
        A_Wv.reshape(d_model * n_heads, d_head),
        jnp.transpose(A_Wo, (0, 2, 1)),
        B_w1,
        B_w3,
        B_w2.T,
    )
    return outT.T[None]
```

```python
import functools

import jax
import jax.numpy as jnp
from jax import lax
import jax.experimental.pallas as pl
import jax.experimental.pallas.tpu as pltpu

F32 = jnp.float32
BF16 = jnp.bfloat16
U32 = jnp.uint32
LANES = 128
LAG = 3
PLAN_WITH_FFN = (1, 2, 8, 2)
PLAN_ALONE = (2, 5, 16, 2)
IN_FLIGHT = 2
TOK_BLOCK = 128
EARLY_BLOCKS = 2
NT_DIMS = (((1,), (1,)), ((), ()))


def _layernorm(x):
    mean = jnp.mean(x, axis=-1, keepdims=True)
    xc = x - mean
    var = jnp.mean(xc * xc, axis=-1, keepdims=True)
    return xc * lax.rsqrt(var + 1e-5)


def _pack(x):
    return pltpu.bitcast(x.astype(BF16), U32)


def _load_slabs(ref, first, count, n_rows=None, width=None, row0=0):
    words = slice(row0 // 2, ref.shape[1] if n_rows is None else (row0 + n_rows) // 2)
    lanes = [LANES] * count
    if width is not None and width % LANES:
        lanes[-1] = width % LANES
    parts = [pltpu.bitcast(ref[first + i, words, 0:lanes[i]], BF16) for i in range(count)]
    return parts[0] if count == 1 else jnp.concatenate(parts, axis=1)


def _store_slabs(ref, row0, value):
    words = _pack(value)
    n_rows, width = words.shape
    for i in range(pl.cdiv(width, LANES)):
        part = words[:, i * LANES:min(width, (i + 1) * LANES)]
        ref[i, row0 // 2:row0 // 2 + n_rows, 0:part.shape[1]] = part


def _kernel(xT_hbm, mem0_ref, wq_hbm, wk_hbm, wv_hbm, woT_hbm, w1_hbm, w3_hbm, w2T_hbm,
            outT_hbm,
            qkv_stage, wqkv, woT, w1, w3, w2T, xT, xs, outs,
            h_att, h_ffn, o_scr, act, res_ffn, res_att, x2_buf, pending, fill_scr, sems,
            *, seg, n_mem):
    seq, d_model = xs.shape
    n_heads, _, d_head = woT.shape
    n_ff = w1.shape[0]
    n_dm = h_att.shape[0]
    n_seg = seq // seg
    m2 = 2 * n_mem
    rows = m2 + 2 * seg
    scale = d_head ** -0.5
    d_main = d_model // LANES * LANES

    n_blk = seq // TOK_BLOCK

    def block(b):
        if isinstance(b, int):
            return pl.ds(b * TOK_BLOCK, TOK_BLOCK)
        return pl.ds(pl.multiple_of(b * TOK_BLOCK, TOK_BLOCK), TOK_BLOCK)

    def slab_copies(src, dst, sem):
        words = src.bitcast(U32)
        return [pltpu.make_async_copy(words.at[:, pl.ds(c * LANES, LANES)], dst.at[c], sem)
                for c in range(n_ff)]

    def x_copies(blocks, sem):
        return [pltpu.make_async_copy(xT_hbm.at[:, block(b)], xT.at[b], sem) for b in blocks]

    def out_copies(blocks, sem):
        return [pltpu.make_async_copy(xT.at[b], outT_hbm.at[:, block(b)], sem) for b in blocks]

    loads = [
        x_copies(range(EARLY_BLOCKS), sems.at[0]),
        [pltpu.make_async_copy(wq_hbm, qkv_stage.at[0], sems.at[1])],
        [pltpu.make_async_copy(wk_hbm, qkv_stage.at[1], sems.at[2])],
        [pltpu.make_async_copy(wv_hbm, qkv_stage.at[2], sems.at[3])],
        [pltpu.make_async_copy(woT_hbm.bitcast(U32), woT, sems.at[4])],
        slab_copies(w1_hbm, w1, sems.at[5]),
        slab_copies(w3_hbm, w3, sems.at[6]),
        slab_copies(w2T_hbm, w2T, sems.at[7]),
        x_copies(range(EARLY_BLOCKS, n_blk), sems.at[8]),
    ]

    def start_load(i):
        if i < len(loads):
            for c in loads[i]:
                c.start()

    def finish_load(i):
        for c in loads[i]:
            c.wait()
        start_load(i + IN_FLIGHT)

    for i in range(IN_FLIGHT):
        start_load(i)

    ri = lax.broadcasted_iota(jnp.int32, (rows, rows), 0)
    ci = lax.broadcasted_iota(jnp.int32, (rows, rows), 1)

    def layer_of(i):
        return jnp.where(i < m2, i // n_mem, (i - m2) // seg)

    def pos_of(i):
        return jnp.where(i < m2, i % n_mem, n_mem + (i - m2) % seg)

    visible = (pos_of(ri) < n_mem) | (pos_of(ri) >= pos_of(ci))
    fill_scr[...] = jnp.where(layer_of(ri) == layer_of(ci),
                              jnp.where(visible, 0.0, -1e9), -jnp.inf).astype(F32)

    def transpose_in(b):
        xs[block(b), :] = xT[b].astype(F32).T.astype(BF16)

    def transpose_out(b):
        xT[b] = outs[block(b), :].astype(F32).T.astype(BF16)

    finish_load(0)
    for b in range(EARLY_BLOCKS):
        transpose_in(b)
    mem0 = mem0_ref[...].astype(F32)
    _store_slabs(h_att, 0, jnp.concatenate([mem0, mem0], axis=0))
    _store_slabs(h_att, m2, _layernorm(xs[0:seg, :].astype(F32)))

    for i in range(3):
        finish_load(1 + i)

        def regroup(blk, carry, i=i):
            src = pl.ds(pl.multiple_of(blk * (16 * n_heads), 16 * n_heads), 16 * n_heads)
            u = pltpu.bitcast(qkv_stage[i, src, :], U32).reshape(8, 2, n_heads // 2, d_head)
            even = jnp.swapaxes(u[:, 0], 0, 1)
            odd = jnp.swapaxes(u[:, 1], 0, 1)
            lo = (even & jnp.uint32(0xFFFF)) | (odd << 16)
            hi = (even >> 16) | (odd & jnp.uint32(0xFFFF0000))
            dst = pl.ds(pl.multiple_of(blk * 8, 8), 8)
            for h in range(n_heads):
                wqkv[3 * h + i, dst, :] = (lo, hi)[h % 2][h // 2]
            return carry

        lax.fori_loop(0, d_model // 16, regroup, 0)

    def seg_rows(s):
        if isinstance(s, int):
            return pl.ds(s * seg, seg)
        return pl.ds(pl.multiple_of(s * seg, seg), seg)

    def x_seg(s):
        return xs[seg_rows(s), :].astype(F32)

    def project(hd, n):
        h = _load_slabs(h_att, 0, n_dm, n, d_model)
        qkv = jnp.dot(h, _load_slabs(wqkv, 3 * hd, 3), preferred_element_type=F32).astype(BF16)
        return tuple(qkv[:, i * d_head:(i + 1) * d_head] for i in range(3))

    def scores(q, k):
        n = q.shape[0]
        s = lax.dot_general(q, k, NT_DIMS, preferred_element_type=F32)
        fill = fill_scr[0:n, 0:n]
        s = jnp.where(fill == 0.0, s * scale, fill)
        e = jnp.exp(s - jnp.max(s, axis=-1, keepdims=True))
        total = jnp.sum(e, axis=-1, keepdims=True)
        inv = pl.reciprocal(total, approx=True)
        inv = inv * (2.0 - total * inv)
        return (e * inv).astype(BF16)

    def ffn_up(c, n, row0=0):
        h = _load_slabs(h_ffn, 0, n_dm, n, d_model)
        w = jnp.concatenate([_load_slabs(w1, c, 1), _load_slabs(w3, c, 1)], axis=1)
        gate_up = jnp.dot(h, w, preferred_element_type=F32)
        half = 0.5 * gate_up[:, :LANES]
        act[c, row0 // 2:(row0 + n) // 2, :] = _pack((half * jnp.tanh(half) + half) * gate_up[:, LANES:])

    def contract(lhs, rhs, first, count, n, n_out=None, row0=0):
        return lax.dot_general(_load_slabs(lhs, first, count, n, row0=row0),
                               _load_slabs(rhs, first, count, n_out),
                               NT_DIMS, preferred_element_type=F32)

    def contract_rest(lhs, rhs, first, count, n):
        return lax.dot_general(_load_slabs(rhs, first, count, d_model - d_main, row0=d_main),
                               _load_slabs(lhs, first, count, n),
                               NT_DIMS, preferred_element_type=F32)

    def mix(n_att, n_ffn, act_row0=0, before_proj=None, side_work=()):
        qk_delay, pv_delay, n_chunks, spacing = PLAN_WITH_FFN if n_ffn else PLAN_ALONE
        qkv, probs = {}, {}
        side_work = list(side_work)

        def attention_slot(i):
            if 0 <= i - qk_delay < n_heads:
                q, k, _ = qkv[i - qk_delay]
                probs[i - qk_delay] = scores(q, k)
            if 0 <= i - pv_delay < n_heads:
                hd = i - pv_delay
                o = jnp.dot(probs.pop(hd), qkv.pop(hd)[2], preferred_element_type=F32)
                o_scr[hd, 0:n_att // 2, :] = _pack(o)

        ff_done = 0
        for i in range(n_heads):
            qkv[i] = project(i, n_att)
            while n_ffn and ff_done < (i + 1) * n_ff // n_heads:
                ffn_up(ff_done, n_ffn, act_row0)
                ff_done += 1
            attention_slot(i)
            if side_work:
                side_work.pop(0)()
        if before_proj is not None:
            before_proj()
        per = n_heads // n_chunks
        assert pv_delay * spacing * per <= n_heads - pv_delay
        split = n_att > d_model - d_main
        a = rest = None
        for c in range(n_chunks):
            part = contract(o_scr, woT, c * per, per, n_att, d_main if split else None)
            a = part if a is None else a + part
            if split:
                part = contract_rest(o_scr, woT, c * per, per, n_att)
                rest = part if rest is None else rest + part
            if (c + 1) % spacing == 0:
                attention_slot(n_heads + c // spacing)
        return jnp.concatenate([a, rest.T], axis=1) if split else a

    def ffn_down(n):
        return res_ffn[0:n, :] + contract(act, w2T, 0, n_ff, n)

    def queue_ffn(slot, x):
        res_ffn[slot * seg:(slot + 1) * seg, :] = x
        _store_slabs(h_ffn, slot * seg, _layernorm(x))

    def set_memory(first, second):
        _store_slabs(h_att, 0, jnp.concatenate([first, second], axis=0))

    one = m2 + seg

    for t in range(LAG):
        last = t == LAG - 1
        if last:
            finish_load(5)
            finish_load(6)
        a = mix(one, 2 * seg if last else 0,
                before_proj=functools.partial(finish_load, 4) if t == 0 else None)
        set_memory(a[0:n_mem], mem0)
        _store_slabs(h_att, m2, _layernorm(x_seg(t + 1)))
        if last:
            finish_load(7)
            y = ffn_down(2 * seg)
            res_att[...] = y[:seg]
            _store_slabs(h_att, one, _layernorm(y[:seg]))
            x2_buf[...] = y[seg:]
        queue_ffn(t % 2, x_seg(t) + a[m2:])

    def advance(t, a, x2):
        x1 = x_seg(t) + a[m2:one]
        x3 = res_att[...] + a[one:]
        set_memory(a[0:n_mem], a[n_mem:m2])
        nxt = min(t + 1, n_seg - 1) if isinstance(t, int) else jnp.minimum(t + 1, n_seg - 1)
        _store_slabs(h_att, m2, _layernorm(x_seg(nxt)))
        res_att[...] = x2
        _store_slabs(h_att, one, _layernorm(x2))
        return x1, x3

    x1, x3 = advance(LAG, mix(rows, seg), x2_buf[...])
    x2_buf[...] = ffn_down(seg)
    queue_ffn(0, x1)
    queue_ffn(1, x3)
    finish_load(8)

    def body(p, carry):
        t = LAG + 1 + 2 * p
        n = 2 * seg
        x1, x3 = advance(t, mix(rows, n), x2_buf[...])
        pending[:, 0:d_main] = res_ffn[0:n, 0:d_main] + contract(act, w2T, 0, n_ff, n, d_main)
        pending[:, d_main:] = res_ffn[0:n, d_main:]
        queue_ffn(0, x1)
        queue_ffn(1, x3)
        transpose_in(jnp.minimum(EARLY_BLOCKS + p, n_blk - 1))

        a = mix(rows, n, act_row0=n)
        rest = contract_rest(act, w2T, 0, n_ff, 2 * n).T
        y = jnp.concatenate([pending[:, 0:d_main], pending[:, d_main:] + rest[0:n]], axis=1)
        outs[seg_rows(t - 1 - LAG), :] = y[seg:].astype(BF16)
        x1, x3 = advance(t + 1, a, y[:seg])
        y = res_ffn[0:n, :] + jnp.concatenate(
            [contract(act, w2T, 0, n_ff, n, d_main, row0=n), rest[n:]], axis=1)
        x2_buf[...] = y[:seg]
        outs[seg_rows(t - LAG), :] = y[seg:].astype(BF16)
        queue_ffn(0, x1)
        queue_ffn(1, x3)
        return carry

    lax.fori_loop(0, (n_seg - LAG - 1) // 2, body, 0)

    done_blk = (n_seg - 1 - LAG) * seg // TOK_BLOCK
    out_early = out_copies(range(done_blk), sems.at[0])
    out_late = out_copies(range(done_blk, n_blk), sems.at[1])

    mem = _load_slabs(h_att, 0, n_dm, m2, d_model).astype(F32)[n_mem:m2]
    x2 = res_att[...]
    for i in range(LAG):
        set_memory(mem, mem)
        _store_slabs(h_att, m2, _layernorm(x2))
        if i == 0:
            a = mix(one, 2 * seg)
            y = ffn_down(2 * seg)
            outs[seg_rows(n_seg - 1 - LAG), :] = y[seg:].astype(BF16)
            upcoming = [x2_buf[...], y[:seg]]
        elif i == 1:
            a = mix(one, 0, side_work=[functools.partial(transpose_out, b) for b in range(done_blk)])
            for c in out_early:
                c.start()
        else:
            a = mix(one, 0)
        queue_ffn(i, x2 + a[m2:])
        mem = a[0:n_mem]
        if upcoming:
            x2 = upcoming.pop(0)
    for c in range(n_ff):
        ffn_up(c, LAG * seg)
    outs[(n_seg - LAG) * seg:, :] = ffn_down(LAG * seg).astype(BF16)
    for b in range(done_blk, n_blk):
        transpose_out(b)
    for c in out_late:
        c.start()
    for c in out_early + out_late:
        c.wait()


@functools.partial(jax.jit, static_argnames=("A_seg_len",))
def pallas_interleave_layers__memory_aug_recurrent_mem_tr__glu_gated_swiglu__prompt_kernel(
    A_x: jax.Array,
    A_mem0: jax.Array,
    A_Wq: jax.Array,
    A_Wk: jax.Array,
    A_Wv: jax.Array,
    A_Wo: jax.Array,
    A_seg_len: int,
    B_x: jax.Array,
    B_w1: jax.Array,
    B_w3: jax.Array,
    B_w2: jax.Array,
):
    del B_x
    batch, seq, d_model = A_x.shape
    _, n_heads, d_head = A_Wq.shape
    n_mem = A_mem0.shape[1]
    d_ff = B_w1.shape[1]
    seg = int(A_seg_len)
    assert batch == 1 and seq % seg == 0 and seq % TOK_BLOCK == 0
    assert d_head == LANES and d_ff % LANES == 0 and (seq // seg - LAG - 1) % 2 == 0
    rows = 2 * (n_mem + seg)
    n_ff = d_ff // LANES
    n_dm = pl.cdiv(d_model, LANES)

    hbm = pl.BlockSpec(memory_space=pl.ANY)
    outT = pl.pallas_call(
        functools.partial(_kernel, seg=seg, n_mem=n_mem),
        out_shape=jax.ShapeDtypeStruct((d_model, seq), A_x.dtype),
        in_specs=[hbm, pl.BlockSpec(memory_space=pltpu.VMEM)] + [hbm] * 7,
        out_specs=hbm,
        scratch_shapes=[
            pltpu.VMEM((3, d_model * n_heads, d_head), BF16),
            pltpu.VMEM((3 * n_heads, d_model // 2, d_head), U32),
            pltpu.VMEM((n_heads, d_model // 2, d_head), U32),
            pltpu.VMEM((n_ff, d_model // 2, LANES), U32),
            pltpu.VMEM((n_ff, d_model // 2, LANES), U32),
            pltpu.VMEM((n_ff, d_model // 2, LANES), U32),
            pltpu.VMEM((seq // TOK_BLOCK, d_model, TOK_BLOCK), BF16),
            pltpu.VMEM((seq, d_model), BF16),
            pltpu.VMEM((seq, d_model), BF16),
            pltpu.VMEM((n_dm, rows // 2, LANES), U32),
            pltpu.VMEM((n_dm, LAG * seg // 2, LANES), U32),
            pltpu.VMEM((n_heads, rows // 2, d_head), U32),
            pltpu.VMEM((n_ff, 2 * seg, LANES), U32),
            pltpu.VMEM((LAG * seg, d_model), F32),
            pltpu.VMEM((seg, d_model), F32),
            pltpu.VMEM((seg, d_model), F32),
            pltpu.VMEM((2 * seg, d_model), F32),
            pltpu.VMEM((rows, rows), F32),
            pltpu.SemaphoreType.DMA((9,)),
        ],
        compiler_params=pltpu.CompilerParams(vmem_limit_bytes=100 * 1024 * 1024),
    )(
        A_x[0].T,
        A_mem0[0],
        A_Wq.reshape(d_model * n_heads, d_head),
        A_Wk.reshape(d_model * n_heads, d_head),
        A_Wv.reshape(d_model * n_heads, d_head),
        jnp.transpose(A_Wo, (0, 2, 1)),
        B_w1,
        B_w3,
        B_w2.T,
    )
    return outT.T[None]
```

```python
import functools

import jax
import jax.numpy as jnp
from jax import lax
import jax.experimental.pallas as pl
import jax.experimental.pallas.tpu as pltpu

F32 = jnp.float32
BF16 = jnp.bfloat16
U32 = jnp.uint32
LANES = 128
LAG = 3
PLAN_WITH_FFN = (1, 2, 8, 2)
PLAN_ALONE = (2, 5, 16, 2)
IN_FLIGHT = 2
TOK_BLOCK = 128
EARLY_BLOCKS = 2
UNTRANSPOSE = False
NT_DIMS = (((1,), (1,)), ((), ()))


def _layernorm(x):
    mean = jnp.mean(x, axis=-1, keepdims=True)
    xc = x - mean
    var = jnp.mean(xc * xc, axis=-1, keepdims=True)
    return xc * lax.rsqrt(var + 1e-5)


def _pack(x):
    return pltpu.bitcast(x.astype(BF16), U32)


def _load_slabs(ref, first, count, n_rows=None, width=None, row0=0):
    words = slice(row0 // 2, ref.shape[1] if n_rows is None else (row0 + n_rows) // 2)
    lanes = [LANES] * count
    if width is not None and width % LANES:
        lanes[-1] = width % LANES
    parts = [pltpu.bitcast(ref[first + i, words, 0:lanes[i]], BF16) for i in range(count)]
    return parts[0] if count == 1 else jnp.concatenate(parts, axis=1)


def _store_slabs(ref, row0, value):
    words = _pack(value)
    n_rows, width = words.shape
    for i in range(pl.cdiv(width, LANES)):
        part = words[:, i * LANES:min(width, (i + 1) * LANES)]
        ref[i, row0 // 2:row0 // 2 + n_rows, 0:part.shape[1]] = part


def _kernel(xT_hbm, mem0_ref, wq_hbm, wk_hbm, wv_hbm, woT_hbm, w1_hbm, w3_hbm, w2T_hbm,
            outT_hbm,
            qkv_stage, wqkv, woT, w1, w3, w2T, wo_main, w2_main, xT, xs, outs,
            h_att, h_ffn, o_scr, act, res_ffn, res_att, x2_buf, pending, fill_scr, sems,
            *, seg, n_mem):
    seq, d_model = xs.shape
    n_heads, _, d_head = woT.shape
    n_ff = w1.shape[0]
    n_dm = h_att.shape[0]
    n_seg = seq // seg
    m2 = 2 * n_mem
    rows = m2 + 2 * seg
    scale = d_head ** -0.5
    d_main = d_model // LANES * LANES
    n_main = d_main // LANES
    lhs_rows = (rows, 2 * seg)

    n_blk = seq // TOK_BLOCK

    def block(b):
        if isinstance(b, int):
            return pl.ds(b * TOK_BLOCK, TOK_BLOCK)
        return pl.ds(pl.multiple_of(b * TOK_BLOCK, TOK_BLOCK), TOK_BLOCK)

    def slab_copies(src, dst, sem):
        words = src.bitcast(U32)
        return [pltpu.make_async_copy(words.at[:, pl.ds(c * LANES, LANES)], dst.at[c], sem)
                for c in range(n_ff)]

    def x_copies(blocks, sem):
        return [pltpu.make_async_copy(xT_hbm.at[:, block(b)], xT.at[b], sem) for b in blocks]

    def out_copies(blocks, sem):
        return [pltpu.make_async_copy(xT.at[b], outT_hbm.at[:, block(b)], sem) for b in blocks]

    loads = [
        x_copies(range(EARLY_BLOCKS), sems.at[0]),
        [pltpu.make_async_copy(wq_hbm, qkv_stage.at[0], sems.at[1])],
        [pltpu.make_async_copy(wk_hbm, qkv_stage.at[1], sems.at[2])],
        [pltpu.make_async_copy(wv_hbm, qkv_stage.at[2], sems.at[3])],
        [pltpu.make_async_copy(woT_hbm.bitcast(U32), woT, sems.at[4])],
        slab_copies(w1_hbm, w1, sems.at[5]),
        slab_copies(w3_hbm, w3, sems.at[6]),
        slab_copies(w2T_hbm, w2T, sems.at[7]),
        x_copies(range(EARLY_BLOCKS, n_blk), sems.at[8]),
    ]

    def start_load(i):
        if i < len(loads):
            for c in loads[i]:
                c.start()

    def finish_load(i):
        for c in loads[i]:
            c.wait()
        start_load(i + IN_FLIGHT)

    for i in range(IN_FLIGHT):
        start_load(i)

    ri = lax.broadcasted_iota(jnp.int32, (rows, rows), 0)
    ci = lax.broadcasted_iota(jnp.int32, (rows, rows), 1)

    def layer_of(i):
        return jnp.where(i < m2, i // n_mem, (i - m2) // seg)

    def pos_of(i):
        return jnp.where(i < m2, i % n_mem, n_mem + (i - m2) % seg)

    visible = (pos_of(ri) < n_mem) | (pos_of(ri) >= pos_of(ci))
    fill_scr[...] = jnp.where(layer_of(ri) == layer_of(ci),
                              jnp.where(visible, 0.0, -1e9), -jnp.inf).astype(F32)

    def transpose_in(b):
        xs[block(b), :] = xT[b].astype(F32).T.astype(BF16)

    def transpose_out(b):
        xT[b] = outs[block(b), :].astype(F32).T.astype(BF16)

    finish_load(0)
    for b in range(EARLY_BLOCKS):
        transpose_in(b)
    mem0 = mem0_ref[...].astype(F32)
    _store_slabs(h_att, 0, jnp.concatenate([mem0, mem0], axis=0))
    _store_slabs(h_att, m2, _layernorm(xs[0:seg, :].astype(F32)))

    for i in range(3):
        finish_load(1 + i)

        def regroup(blk, carry, i=i):
            src = pl.ds(pl.multiple_of(blk * (16 * n_heads), 16 * n_heads), 16 * n_heads)
            u = pltpu.bitcast(qkv_stage[i, src, :], U32).reshape(8, 2, n_heads // 2, d_head)
            even = jnp.swapaxes(u[:, 0], 0, 1)
            odd = jnp.swapaxes(u[:, 1], 0, 1)
            lo = (even & jnp.uint32(0xFFFF)) | (odd << 16)
            hi = (even >> 16) | (odd & jnp.uint32(0xFFFF0000))
            dst = pl.ds(pl.multiple_of(blk * 8, 8), 8)
            for h in range(n_heads):
                wqkv[3 * h + i, dst, :] = (lo, hi)[h % 2][h // 2]
            return carry

        lax.fori_loop(0, d_model // 16, regroup, 0)

    def seg_rows(s):
        if isinstance(s, int):
            return pl.ds(s * seg, seg)
        return pl.ds(pl.multiple_of(s * seg, seg), seg)

    def x_seg(s):
        return xs[seg_rows(s), :].astype(F32)

    def project(hd, n):
        h = _load_slabs(h_att, 0, n_dm, n, d_model)
        qkv = jnp.dot(h, _load_slabs(wqkv, 3 * hd, 3), preferred_element_type=F32).astype(BF16)
        return tuple(qkv[:, i * d_head:(i + 1) * d_head] for i in range(3))

    def scores(q, k):
        n = q.shape[0]
        s = lax.dot_general(q, k, NT_DIMS, preferred_element_type=F32)
        fill = fill_scr[0:n, 0:n]
        s = jnp.where(fill == 0.0, s * scale, fill)
        e = jnp.exp(s - jnp.max(s, axis=-1, keepdims=True))
        total = jnp.sum(e, axis=-1, keepdims=True)
        inv = pl.reciprocal(total, approx=True)
        inv = inv * (2.0 - total * inv)
        return (e * inv).astype(BF16)

    def ffn_up(c, n, slab0=0):
        h = _load_slabs(h_ffn, 0, n_dm, n, d_model)
        w = jnp.concatenate([_load_slabs(w1, c, 1), _load_slabs(w3, c, 1)], axis=1)
        gate_up = jnp.dot(h, w, preferred_element_type=F32)
        half = 0.5 * gate_up[:, :LANES]
        act[slab0 + c, 0:n // 2, :] = _pack((half * jnp.tanh(half) + half) * gate_up[:, LANES:])

    def contract(lhs, rhs, first, count, n):
        return lax.dot_general(_load_slabs(lhs, first, count, n), _load_slabs(rhs, first, count),
                               NT_DIMS, preferred_element_type=F32)

    def contract_main(lhs, rhs_t, rhs, first, count, lhs_first):
        x = _load_slabs(lhs, lhs_first, count, lhs_rows[lhs is act])
        if not UNTRANSPOSE:
            return lax.dot_general(x, _load_slabs(rhs_t, first, count, d_main),
                                   NT_DIMS, preferred_element_type=F32)
        w = jnp.concatenate([_load_slabs(rhs, k * n_main, n_main) for k in range(first, first + count)], axis=0)
        return jnp.dot(x, w, preferred_element_type=F32)

    def untranspose(src, dst, k):
        words = _pack(_load_slabs(src, k, 1, d_main).T)
        for j in range(n_main):
            dst[k * n_main + j] = words[:, j * LANES:(j + 1) * LANES]

    def contract_rest(x, rhs, first, count):
        return lax.dot_general(_load_slabs(rhs, first, count, d_model - d_main, row0=d_main), x,
                               NT_DIMS, preferred_element_type=F32)

    def mix(n_att, n_ffn, act_slab0=0, split=False, before_proj=None, side_work=()):
        qk_delay, pv_delay, n_chunks, spacing = PLAN_WITH_FFN if n_ffn else PLAN_ALONE
        qkv, probs = {}, {}
        side_work = list(side_work)

        def attention_slot(i):
            if 0 <= i - qk_delay < n_heads:
                q, k, _ = qkv[i - qk_delay]
                probs[i - qk_delay] = scores(q, k)
            if 0 <= i - pv_delay < n_heads:
                hd = i - pv_delay
                o = jnp.dot(probs.pop(hd), qkv.pop(hd)[2], preferred_element_type=F32)
                o_scr[hd, 0:n_att // 2, :] = _pack(o)

        ff_done = 0
        for i in range(n_heads):
            qkv[i] = project(i, n_att)
            while n_ffn and ff_done < (i + 1) * n_ff // n_heads:
                ffn_up(ff_done, n_ffn, act_slab0)
                ff_done += 1
            attention_slot(i)
            if side_work:
                side_work.pop(0)()
        if before_proj is not None:
            before_proj()
        per = n_heads // n_chunks
        assert pv_delay * spacing * per <= n_heads - pv_delay
        a = rest = None
        for c in range(n_chunks):
            part = (contract_main(o_scr, woT, wo_main, c * per, per, c * per) if split
                    else contract(o_scr, woT, c * per, per, n_att))
            a = part if a is None else a + part
            if split:
                part = contract_rest(_load_slabs(o_scr, c * per, per, n_att), woT, c * per, per)
                rest = part if rest is None else rest + part
            if (c + 1) % spacing == 0:
                attention_slot(n_heads + c // spacing)
        return jnp.concatenate([a, rest.T], axis=1) if split else a

    def ffn_down(n):
        return res_ffn[0:n, :] + contract(act, w2T, 0, n_ff, n)

    def queue_ffn(slot, x):
        res_ffn[slot * seg:(slot + 1) * seg, :] = x
        _store_slabs(h_ffn, slot * seg, _layernorm(x))

    def set_memory(first, second):
        _store_slabs(h_att, 0, jnp.concatenate([first, second], axis=0))

    one = m2 + seg

    for t in range(LAG):
        last = t == LAG - 1
        if last:
            finish_load(5)
            finish_load(6)
        a = mix(one, 2 * seg if last else 0,
                before_proj=functools.partial(finish_load, 4) if t == 0 else None)
        set_memory(a[0:n_mem], mem0)
        _store_slabs(h_att, m2, _layernorm(x_seg(t + 1)))
        if last:
            finish_load(7)
            y = ffn_down(2 * seg)
            res_att[...] = y[:seg]
            _store_slabs(h_att, one, _layernorm(y[:seg]))
            x2_buf[...] = y[seg:]
        queue_ffn(t % 2, x_seg(t) + a[m2:])

    def advance(t, a, x2):
        x1 = x_seg(t) + a[m2:one]
        x3 = res_att[...] + a[one:]
        set_memory(a[0:n_mem], a[n_mem:m2])
        nxt = min(t + 1, n_seg - 1) if isinstance(t, int) else jnp.minimum(t + 1, n_seg - 1)
        _store_slabs(h_att, m2, _layernorm(x_seg(nxt)))
        res_att[...] = x2
        _store_slabs(h_att, one, _layernorm(x2))
        return x1, x3

    def untranspose_share(i):
        untranspose(woT, wo_main, i)
        for c in range(i * n_ff // n_heads, (i + 1) * n_ff // n_heads):
            untranspose(w2T, w2_main, c)

    a = mix(rows, seg, side_work=[functools.partial(untranspose_share, i) for i in range(n_heads if UNTRANSPOSE else 0)])
    x1, x3 = advance(LAG, a, x2_buf[...])
    n_pass = 2 * seg
    half_ff = n_ff // 2
    pending[0:seg, :] = ffn_down(seg)
    pending[seg:, :] = jnp.zeros((seg, d_model), F32)
    for c in range(n_ff):
        act[n_ff + c] = jnp.zeros(act.shape[1:], U32)
    queue_ffn(0, x1)
    queue_ffn(1, x3)
    finish_load(8)

    def body(i, carry):
        t = LAG + 1 + i
        odd = i % 2
        a = mix(rows, n_pass, act_slab0=odd * n_ff, split=True)
        both = jnp.concatenate([_load_slabs(act, j * n_ff + odd * half_ff, half_ff, n_pass)
                                for j in range(2)], axis=0)
        rest = contract_rest(both, w2T, odd * half_ff, half_ff).T
        rest_now = jnp.where(odd == 1, rest[n_pass:], rest[:n_pass])
        rest_prev = jnp.where(odd == 1, rest[:n_pass], rest[n_pass:])
        y = jnp.concatenate([pending[:, 0:d_main], pending[:, d_main:] + rest_prev], axis=1)
        outs[seg_rows(jnp.maximum(t - 2 - LAG, 0)), :] = y[seg:].astype(BF16)
        x1, x3 = advance(t, a, y[:seg])
        pending[:, 0:d_main] = (res_ffn[0:n_pass, 0:d_main]
                                + contract_main(act, w2T, w2_main, 0, n_ff, odd * n_ff))
        pending[:, d_main:] = res_ffn[0:n_pass, d_main:] + rest_now
        queue_ffn(0, x1)
        queue_ffn(1, x3)
        transpose_in(jnp.minimum(EARLY_BLOCKS + i, n_blk - 1))
        return carry

    n_steady = n_seg - LAG - 1
    lax.fori_loop(0, n_steady, body, 0)
    odd = n_steady % 2
    last_act = _load_slabs(act, (1 - odd) * n_ff + odd * half_ff, half_ff, n_pass)
    rest = contract_rest(last_act, w2T, odd * half_ff, half_ff).T
    y = jnp.concatenate([pending[:, 0:d_main], pending[:, d_main:] + rest], axis=1)
    x2_buf[...] = y[:seg]
    outs[seg_rows(n_seg - 2 - LAG), :] = y[seg:].astype(BF16)

    done_blk = (n_seg - 1 - LAG) * seg // TOK_BLOCK
    out_early = out_copies(range(done_blk), sems.at[0])
    out_late = out_copies(range(done_blk, n_blk), sems.at[1])

    mem = _load_slabs(h_att, 0, n_dm, m2, d_model).astype(F32)[n_mem:m2]
    x2 = res_att[...]
    for i in range(LAG):
        set_memory(mem, mem)
        _store_slabs(h_att, m2, _layernorm(x2))
        if i == 0:
            a = mix(one, 2 * seg)
            y = ffn_down(2 * seg)
            outs[seg_rows(n_seg - 1 - LAG), :] = y[seg:].astype(BF16)
            upcoming = [x2_buf[...], y[:seg]]
        elif i == 1:
            a = mix(one, 0, side_work=[functools.partial(transpose_out, b) for b in range(done_blk)])
            for c in out_early:
                c.start()
        else:
            a = mix(one, 0)
        queue_ffn(i, x2 + a[m2:])
        mem = a[0:n_mem]
        if upcoming:
            x2 = upcoming.pop(0)
    for c in range(n_ff):
        ffn_up(c, LAG * seg)
    outs[(n_seg - LAG) * seg:, :] = ffn_down(LAG * seg).astype(BF16)
    for b in range(done_blk, n_blk):
        transpose_out(b)
    for c in out_late:
        c.start()
    for c in out_early + out_late:
        c.wait()


@functools.partial(jax.jit, static_argnames=("A_seg_len",))
def pallas_interleave_layers__memory_aug_recurrent_mem_tr__glu_gated_swiglu__prompt_kernel(
    A_x: jax.Array,
    A_mem0: jax.Array,
    A_Wq: jax.Array,
    A_Wk: jax.Array,
    A_Wv: jax.Array,
    A_Wo: jax.Array,
    A_seg_len: int,
    B_x: jax.Array,
    B_w1: jax.Array,
    B_w3: jax.Array,
    B_w2: jax.Array,
):
    del B_x
    batch, seq, d_model = A_x.shape
    _, n_heads, d_head = A_Wq.shape
    n_mem = A_mem0.shape[1]
    d_ff = B_w1.shape[1]
    seg = int(A_seg_len)
    assert batch == 1 and seq % seg == 0 and seq % TOK_BLOCK == 0
    assert d_head == LANES and d_ff % (2 * LANES) == 0
    rows = 2 * (n_mem + seg)
    n_ff = d_ff // LANES
    n_dm = pl.cdiv(d_model, LANES)

    hbm = pl.BlockSpec(memory_space=pl.ANY)
    outT = pl.pallas_call(
        functools.partial(_kernel, seg=seg, n_mem=n_mem),
        out_shape=jax.ShapeDtypeStruct((d_model, seq), A_x.dtype),
        in_specs=[hbm, pl.BlockSpec(memory_space=pltpu.VMEM)] + [hbm] * 7,
        out_specs=hbm,
        scratch_shapes=[
            pltpu.VMEM((3, d_model * n_heads, d_head), BF16),
            pltpu.VMEM((3 * n_heads, d_model // 2, d_head), U32),
            pltpu.VMEM((n_heads, d_model // 2, d_head), U32),
            pltpu.VMEM((n_ff, d_model // 2, LANES), U32),
            pltpu.VMEM((n_ff, d_model // 2, LANES), U32),
            pltpu.VMEM((n_ff, d_model // 2, LANES), U32),
            pltpu.VMEM((n_heads * (d_model // LANES), LANES // 2, LANES), U32),
            pltpu.VMEM((n_ff * (d_model // LANES), LANES // 2, LANES), U32),
            pltpu.VMEM((seq // TOK_BLOCK, d_model, TOK_BLOCK), BF16),
            pltpu.VMEM((seq, d_model), BF16),
            pltpu.VMEM((seq, d_model), BF16),
            pltpu.VMEM((n_dm, rows // 2, LANES), U32),
            pltpu.VMEM((n_dm, LAG * seg // 2, LANES), U32),
            pltpu.VMEM((n_heads, rows // 2, d_head), U32),
            pltpu.VMEM((2 * n_ff, LAG * seg // 2, LANES), U32),
            pltpu.VMEM((LAG * seg, d_model), F32),
            pltpu.VMEM((seg, d_model), F32),
            pltpu.VMEM((seg, d_model), F32),
            pltpu.VMEM((2 * seg, d_model), F32),
            pltpu.VMEM((rows, rows), F32),
            pltpu.SemaphoreType.DMA((9,)),
        ],
        compiler_params=pltpu.CompilerParams(vmem_limit_bytes=100 * 1024 * 1024),
    )(
        A_x[0].T,
        A_mem0[0],
        A_Wq.reshape(d_model * n_heads, d_head),
        A_Wk.reshape(d_model * n_heads, d_head),
        A_Wv.reshape(d_model * n_heads, d_head),
        jnp.transpose(A_Wo, (0, 2, 1)),
        B_w1,
        B_w3,
        B_w2.T,
    )
    return outT.T[None]
```

```python
import functools

import jax
import jax.numpy as jnp
from jax import lax
import jax.experimental.pallas as pl
import jax.experimental.pallas.tpu as pltpu

F32 = jnp.float32
BF16 = jnp.bfloat16
U32 = jnp.uint32
LANES = 128
LAG = 3
PLAN_WITH_FFN = (1, 2, 8, 2)
PLAN_ALONE = (2, 5, 16, 2)
IN_FLIGHT = 2
TOK_BLOCK = 128
EARLY_BLOCKS = 2
PEEL = False
NT_DIMS = (((1,), (1,)), ((), ()))


def _layernorm(x):
    mean = jnp.mean(x, axis=-1, keepdims=True)
    xc = x - mean
    var = jnp.mean(xc * xc, axis=-1, keepdims=True)
    return xc * lax.rsqrt(var + 1e-5)


def _pack(x):
    return pltpu.bitcast(x.astype(BF16), U32)


def _rows(start, size):
    return pl.ds(start if isinstance(start, int) else pl.multiple_of(start, 8), size)


def _load_slabs(ref, first, count, n_rows=None, width=None, row0=0):
    words = slice(row0 // 2, ref.shape[1] if n_rows is None else (row0 + n_rows) // 2)
    lanes = [LANES] * count
    if width is not None and width % LANES:
        lanes[-1] = width % LANES
    parts = [pltpu.bitcast(ref[first + i, words, 0:lanes[i]], BF16) for i in range(count)]
    return parts[0] if count == 1 else jnp.concatenate(parts, axis=1)


def _store_slabs(ref, row0, value):
    words = _pack(value)
    n_rows, width = words.shape
    for i in range(pl.cdiv(width, LANES)):
        part = words[:, i * LANES:min(width, (i + 1) * LANES)]
        ref[i, _rows(row0 // 2, n_rows), 0:part.shape[1]] = part


def _kernel(xT_hbm, mem0_ref, wq_hbm, wk_hbm, wv_hbm, woT_hbm, w1_hbm, w3_hbm, w2T_hbm,
            outT_hbm,
            qkv_stage, wqkv, woT, w1, w3, w2T, xT, xs, outs,
            h_att, h_ffn, o_scr, act, res_ffn, res_att, edge, att_out, pending, fill_scr, sems,
            *, seg, n_mem):
    seq, d_model = xs.shape
    n_heads, _, d_head = woT.shape
    n_ff = w1.shape[0]
    n_dm = h_att.shape[0]
    n_seg = seq // seg
    m2 = 2 * n_mem
    rows = m2 + 2 * seg
    scale = d_head ** -0.5
    d_main = d_model // LANES * LANES

    n_blk = seq // TOK_BLOCK

    def block(b):
        if isinstance(b, int):
            return pl.ds(b * TOK_BLOCK, TOK_BLOCK)
        return pl.ds(pl.multiple_of(b * TOK_BLOCK, TOK_BLOCK), TOK_BLOCK)

    def slab_copies(src, dst, sem):
        words = src.bitcast(U32)
        return [pltpu.make_async_copy(words.at[:, pl.ds(c * LANES, LANES)], dst.at[c], sem)
                for c in range(n_ff)]

    def x_copies(blocks, sem):
        return [pltpu.make_async_copy(xT_hbm.at[:, block(b)], xT.at[b], sem) for b in blocks]

    def out_copies(blocks, sem):
        return [pltpu.make_async_copy(xT.at[b], outT_hbm.at[:, block(b)], sem) for b in blocks]

    loads = [
        x_copies(range(EARLY_BLOCKS), sems.at[0]),
        [pltpu.make_async_copy(wq_hbm, qkv_stage.at[0], sems.at[1])],
        [pltpu.make_async_copy(wk_hbm, qkv_stage.at[1], sems.at[2])],
        [pltpu.make_async_copy(wv_hbm, qkv_stage.at[2], sems.at[3])],
        [pltpu.make_async_copy(woT_hbm.bitcast(U32), woT, sems.at[4])],
        slab_copies(w1_hbm, w1, sems.at[5]),
        slab_copies(w3_hbm, w3, sems.at[6]),
        slab_copies(w2T_hbm, w2T, sems.at[7]),
        x_copies(range(EARLY_BLOCKS, n_blk), sems.at[8]),
    ]

    def start_load(i):
        if i < len(loads):
            for c in loads[i]:
                c.start()

    def finish_load(i):
        for c in loads[i]:
            c.wait()
        start_load(i + IN_FLIGHT)

    for i in range(IN_FLIGHT):
        start_load(i)

    ri = lax.broadcasted_iota(jnp.int32, (rows, rows), 0)
    ci = lax.broadcasted_iota(jnp.int32, (rows, rows), 1)

    def layer_of(i):
        return jnp.where(i < m2, i // n_mem, (i - m2) // seg)

    def pos_of(i):
        return jnp.where(i < m2, i % n_mem, n_mem + (i - m2) % seg)

    visible = (pos_of(ri) < n_mem) | (pos_of(ri) >= pos_of(ci))
    fill_scr[...] = jnp.where(layer_of(ri) == layer_of(ci),
                              jnp.where(visible, 0.0, -1e9), -jnp.inf).astype(F32)

    def transpose_in(b):
        xs[block(b), :] = xT[b].astype(F32).T.astype(BF16)

    def transpose_out(b):
        xT[b] = outs[block(b), :].astype(F32).T.astype(BF16)

    finish_load(0)
    for b in range(EARLY_BLOCKS):
        transpose_in(b)
    mem0 = mem0_ref[...].astype(F32)
    _store_slabs(h_att, 0, jnp.concatenate([mem0, mem0], axis=0))
    _store_slabs(h_att, m2, _layernorm(xs[0:seg, :].astype(F32)))

    for i in range(3):
        finish_load(1 + i)

        def regroup(blk, carry, i=i):
            src = pl.ds(pl.multiple_of(blk * (16 * n_heads), 16 * n_heads), 16 * n_heads)
            u = pltpu.bitcast(qkv_stage[i, src, :], U32).reshape(8, 2, n_heads // 2, d_head)
            even = jnp.swapaxes(u[:, 0], 0, 1)
            odd = jnp.swapaxes(u[:, 1], 0, 1)
            lo = (even & jnp.uint32(0xFFFF)) | (odd << 16)
            hi = (even >> 16) | (odd & jnp.uint32(0xFFFF0000))
            dst = pl.ds(pl.multiple_of(blk * 8, 8), 8)
            for h in range(n_heads):
                wqkv[3 * h + i, dst, :] = (lo, hi)[h % 2][h // 2]
            return carry

        lax.fori_loop(0, d_model // 16, regroup, 0)

    def seg_rows(s):
        return pl.ds(s * seg if isinstance(s, int) else pl.multiple_of(s * seg, seg), seg)

    def x_seg(s):
        return xs[seg_rows(s), :].astype(F32)

    def project(hd, n):
        h = _load_slabs(h_att, 0, n_dm, n, d_model)
        qkv = jnp.dot(h, _load_slabs(wqkv, 3 * hd, 3), preferred_element_type=F32).astype(BF16)
        return tuple(qkv[:, i * d_head:(i + 1) * d_head] for i in range(3))

    def scores(q, k):
        n = q.shape[0]
        s = lax.dot_general(q, k, NT_DIMS, preferred_element_type=F32)
        fill = fill_scr[0:n, 0:n]
        s = jnp.where(fill == 0.0, s * scale, fill)
        e = jnp.exp(s - jnp.max(s, axis=-1, keepdims=True))
        total = jnp.sum(e, axis=-1, keepdims=True)
        inv = pl.reciprocal(total, approx=True)
        inv = inv * (2.0 - total * inv)
        return (e * inv).astype(BF16)

    def ffn_up(c, n, slab0=0):
        h = _load_slabs(h_ffn, 0, n_dm, n, d_model)
        w = jnp.concatenate([_load_slabs(w1, c, 1), _load_slabs(w3, c, 1)], axis=1)
        gate_up = jnp.dot(h, w, preferred_element_type=F32)
        half = 0.5 * gate_up[:, :LANES]
        act[slab0 + c, 0:n // 2, :] = _pack((half * jnp.tanh(half) + half) * gate_up[:, LANES:])

    def contract(lhs, rhs, first, count, n, n_out=None, lhs_offset=0):
        return lax.dot_general(_load_slabs(lhs, lhs_offset + first, count, n),
                               _load_slabs(rhs, first, count, n_out),
                               NT_DIMS, preferred_element_type=F32)

    def contract_rest(x, rhs, first, count):
        return lax.dot_general(_load_slabs(rhs, first, count, d_model - d_main, row0=d_main), x,
                               NT_DIMS, preferred_element_type=F32)

    def mix(n_att, n_ffn, act_slab0=0, split=False, before_proj=None):
        qk_delay, pv_delay, n_chunks, spacing = PLAN_WITH_FFN if n_ffn else PLAN_ALONE
        qkv, probs = {}, {}

        def attention_slot(i):
            if 0 <= i - qk_delay < n_heads:
                q, k, _ = qkv[i - qk_delay]
                probs[i - qk_delay] = scores(q, k)
            if 0 <= i - pv_delay < n_heads:
                hd = i - pv_delay
                o = jnp.dot(probs.pop(hd), qkv.pop(hd)[2], preferred_element_type=F32)
                o_scr[hd, 0:n_att // 2, :] = _pack(o)

        ff_done = 0
        for i in range(n_heads):
            qkv[i] = project(i, n_att)
            while n_ffn and ff_done < (i + 1) * n_ff // n_heads:
                ffn_up(ff_done, n_ffn, act_slab0)
                ff_done += 1
            attention_slot(i)
        if before_proj is not None:
            before_proj()
        per = n_heads // n_chunks
        assert pv_delay * spacing * per <= n_heads - pv_delay
        a = rest = None
        for c in range(n_chunks):
            part = contract(o_scr, woT, c * per, per, n_att, d_main if split else None)
            a = part if a is None else a + part
            if split:
                part = contract_rest(_load_slabs(o_scr, c * per, per, n_att), woT, c * per, per)
                rest = part if rest is None else rest + part
            if (c + 1) % spacing == 0:
                attention_slot(n_heads + c // spacing)
        return jnp.concatenate([a, rest.T], axis=1) if split else a

    def ffn_down(n):
        return res_ffn[0:n, :] + contract(act, w2T, 0, n_ff, n)

    def queue_ffn(slot, x):
        res_ffn[seg_rows(slot), :] = x
        _store_slabs(h_ffn, slot * seg, _layernorm(x))

    def set_memory(first, second):
        _store_slabs(h_att, 0, jnp.concatenate([first, second], axis=0))

    one = m2 + seg

    n_pass = 2 * seg
    half_ff = n_ff // 2
    segs_per_blk = TOK_BLOCK // seg
    done_blk = (n_seg - 1 - LAG) // segs_per_blk
    out_early = out_copies(range(done_blk), sems.at[0])
    out_late = out_copies(range(done_blk, n_blk), sems.at[1])

    def advance(t, a, x2):
        x1 = x_seg(t) + a[m2:one]
        x3 = res_att[...] + a[one:]
        set_memory(a[0:n_mem], a[n_mem:m2])
        _store_slabs(h_att, m2, _layernorm(x_seg(jnp.minimum(t + 1, n_seg - 1))))
        res_att[...] = x2
        _store_slabs(h_att, one, _layernorm(x2))
        return x1, x3

    def completed(rest):
        return jnp.concatenate([pending[:, 0:d_main], pending[:, d_main:] + rest], axis=1)

    def steady_step(t, carry):
        odd = t % 2
        a = mix(rows, n_pass, act_slab0=odd * n_ff, split=True)
        both = jnp.concatenate([_load_slabs(act, j * n_ff + odd * half_ff, half_ff, n_pass)
                                for j in range(2)], axis=0)
        rest = contract_rest(both, w2T, odd * half_ff, half_ff).T
        rest_now = jnp.where(odd == 1, rest[n_pass:], rest[:n_pass])
        y = completed(jnp.where(odd == 1, rest[:n_pass], rest[n_pass:]))
        outs[seg_rows(jnp.maximum(t - 2 - LAG, 0)), :] = y[seg:].astype(BF16)
        x1, x3 = advance(t, a, y[:seg])
        pending[:, 0:d_main] = (res_ffn[0:n_pass, 0:d_main]
                                + contract(act, w2T, 0, n_ff, n_pass, d_main, odd * n_ff))
        pending[:, d_main:] = res_ffn[0:n_pass, d_main:] + rest_now
        queue_ffn(0, x1)
        queue_ffn(1, x3)
        transpose_in(jnp.clip(t - LAG + 1, EARLY_BLOCKS, n_blk - 1))
        transpose_out(jnp.maximum((t - 1 - LAG) // segs_per_blk - 1, 0))
        return carry

    def both_layers():
        x2 = pending[0:seg, :]
        res_att[...] = x2
        _store_slabs(h_att, one, _layernorm(x2))
        first = LAG
        if PEEL:
            x1, x3 = advance(first, mix(rows, seg), pending[seg:, :])
            pending[0:seg, :] = ffn_down(seg)
            queue_ffn(0, x1)
            queue_ffn(1, x3)
            first += 1
        else:
            pending[0:seg, :] = pending[seg:, :]
        for c in range(n_ff):
            act[(1 - first % 2) * n_ff + c] = jnp.zeros(act.shape[1:], U32)
        finish_load(8)
        lax.fori_loop(first, n_seg, steady_step, 0)

        odd = n_seg % 2
        last_act = _load_slabs(act, (1 - odd) * n_ff + odd * half_ff, half_ff, n_pass)
        y = completed(contract_rest(last_act, w2T, odd * half_ff, half_ff).T)
        outs[seg_rows(n_seg - 2 - LAG), :] = y[seg:].astype(BF16)
        for b in range((n_seg - 2 - LAG) // segs_per_blk, done_blk):
            transpose_out(b)
        for c in out_early:
            c.start()
        edge[seg_rows(LAG + 1), :] = res_att[...]
        edge[seg_rows(LAG + 2), :] = y[:seg]
        mem = _load_slabs(h_att, 0, n_dm, m2, d_model).astype(F32)[n_mem:m2]
        set_memory(mem, mem)
        _store_slabs(h_att, m2, _layernorm(res_att[...]))

    def edge_step(e, carry):
        with_ffn = (e == LAG - 1) | (e == LAG)

        @pl.when(jnp.logical_not(with_ffn))
        def _():
            att_out[...] = mix(one, 0, before_proj=lambda: pl.when(e == 0)(lambda: finish_load(4)))

        @pl.when(with_ffn)
        def _():
            @pl.when(e == LAG - 1)
            def _():
                finish_load(5)
                finish_load(6)

            att_out[...] = mix(one, n_pass)
            pl.when(e == LAG - 1)(lambda: finish_load(7))
            pending[...] = ffn_down(n_pass)

        @pl.when(e == LAG)
        def _():
            edge[seg_rows(2 * LAG), :] = pending[0:seg, :]
            outs[seg_rows(n_seg - 1 - LAG), :] = pending[seg:, :].astype(BF16)

        cur = jnp.where(e < LAG, e, e + 1)
        set_memory(att_out[0:n_mem, :], mem0_ref[...].astype(F32))
        _store_slabs(h_att, m2, _layernorm(edge[seg_rows(cur + 1), :]))
        queue_ffn(jnp.where(e < LAG, e % 2, e - LAG), edge[seg_rows(cur), :] + att_out[m2:, :])
        pl.when(e == LAG - 1)(both_layers)
        return carry

    n_fill = (LAG + 1) * seg
    edge[0:n_fill, :] = xs[0:n_fill, :].astype(F32)
    edge[n_fill:, :] = jnp.zeros((n_fill, d_model), F32)
    outs[block(0), :] = jnp.zeros((TOK_BLOCK, d_model), BF16)
    lax.fori_loop(0, 2 * LAG, edge_step, 0)

    for c in range(n_ff):
        ffn_up(c, LAG * seg)
    outs[(n_seg - LAG) * seg:, :] = ffn_down(LAG * seg).astype(BF16)
    for b in range(done_blk, n_blk):
        transpose_out(b)
    for c in out_late:
        c.start()
    for c in out_early + out_late:
        c.wait()


@functools.partial(jax.jit, static_argnames=("A_seg_len",))
def pallas_interleave_layers__memory_aug_recurrent_mem_tr__glu_gated_swiglu__prompt_kernel(
    A_x: jax.Array,
    A_mem0: jax.Array,
    A_Wq: jax.Array,
    A_Wk: jax.Array,
    A_Wv: jax.Array,
    A_Wo: jax.Array,
    A_seg_len: int,
    B_x: jax.Array,
    B_w1: jax.Array,
    B_w3: jax.Array,
    B_w2: jax.Array,
):
    del B_x
    batch, seq, d_model = A_x.shape
    _, n_heads, d_head = A_Wq.shape
    n_mem = A_mem0.shape[1]
    d_ff = B_w1.shape[1]
    seg = int(A_seg_len)
    assert batch == 1 and seq % seg == 0 and seq % TOK_BLOCK == 0
    assert d_head == LANES and d_ff % (2 * LANES) == 0
    rows = 2 * (n_mem + seg)
    n_ff = d_ff // LANES
    n_dm = pl.cdiv(d_model, LANES)

    hbm = pl.BlockSpec(memory_space=pl.ANY)
    outT = pl.pallas_call(
        functools.partial(_kernel, seg=seg, n_mem=n_mem),
        out_shape=jax.ShapeDtypeStruct((d_model, seq), A_x.dtype),
        in_specs=[hbm, pl.BlockSpec(memory_space=pltpu.VMEM)] + [hbm] * 7,
        out_specs=hbm,
        scratch_shapes=[
            pltpu.VMEM((3, d_model * n_heads, d_head), BF16),
            pltpu.VMEM((3 * n_heads, d_model // 2, d_head), U32),
            pltpu.VMEM((n_heads, d_model // 2, d_head), U32),
            pltpu.VMEM((n_ff, d_model // 2, LANES), U32),
            pltpu.VMEM((n_ff, d_model // 2, LANES), U32),
            pltpu.VMEM((n_ff, d_model // 2, LANES), U32),
            pltpu.VMEM((seq // TOK_BLOCK, d_model, TOK_BLOCK), BF16),
            pltpu.VMEM((seq, d_model), BF16),
            pltpu.VMEM((seq, d_model), BF16),
            pltpu.VMEM((n_dm, rows // 2, LANES), U32),
            pltpu.VMEM((n_dm, LAG * seg // 2, LANES), U32),
            pltpu.VMEM((n_heads, rows // 2, d_head), U32),
            pltpu.VMEM((2 * n_ff, LAG * seg // 2, LANES), U32),
            pltpu.VMEM((LAG * seg, d_model), F32),
            pltpu.VMEM((seg, d_model), F32),
            pltpu.VMEM((2 * (LAG + 1) * seg, d_model), F32),
            pltpu.VMEM((rows - seg, d_model), F32),
            pltpu.VMEM((2 * seg, d_model), F32),
            pltpu.VMEM((rows, rows), F32),
            pltpu.SemaphoreType.DMA((9,)),
        ],
        compiler_params=pltpu.CompilerParams(vmem_limit_bytes=100 * 1024 * 1024),
    )(
        A_x[0].T,
        A_mem0[0],
        A_Wq.reshape(d_model * n_heads, d_head),
        A_Wk.reshape(d_model * n_heads, d_head),
        A_Wv.reshape(d_model * n_heads, d_head),
        jnp.transpose(A_Wo, (0, 2, 1)),
        B_w1,
        B_w3,
        B_w2.T,
    )
    return outT.T[None]
```

```python
import functools

import jax
import jax.numpy as jnp
from jax import lax
import jax.experimental.pallas as pl
import jax.experimental.pallas.tpu as pltpu

F32 = jnp.float32
BF16 = jnp.bfloat16
U32 = jnp.uint32
LANES = 128
LAG = 3
PLAN_WITH_FFN = (1, 2, 8, 2)
PLAN_ALONE = (2, 5, 16, 2)
TOK_BLOCK = 128
EARLY_BLOCKS = 2
NT_DIMS = (((1,), (1,)), ((), ()))


def _layernorm(x):
    mean = jnp.mean(x, axis=-1, keepdims=True)
    xc = x - mean
    var = jnp.mean(xc * xc, axis=-1, keepdims=True)
    return xc * lax.rsqrt(var + 1e-5)


def _pack(x):
    return pltpu.bitcast(x.astype(BF16), U32)


def _rows(start, size):
    return pl.ds(start if isinstance(start, int) else pl.multiple_of(start, 8), size)


def _load_slabs(ref, first, count, n_rows=None, width=None, row0=0):
    words = slice(row0 // 2, ref.shape[1] if n_rows is None else (row0 + n_rows) // 2)
    lanes = [LANES] * count
    if width is not None and width % LANES:
        lanes[-1] = width % LANES
    parts = [pltpu.bitcast(ref[first + i, words, 0:lanes[i]], BF16) for i in range(count)]
    return parts[0] if count == 1 else jnp.concatenate(parts, axis=1)


def _store_slabs(ref, row0, value):
    words = _pack(value)
    n_rows, width = words.shape
    for i in range(pl.cdiv(width, LANES)):
        part = words[:, i * LANES:min(width, (i + 1) * LANES)]
        ref[i, _rows(row0 // 2, n_rows), 0:part.shape[1]] = part


def _kernel(xT_hbm, mem0_ref, wq_hbm, wk_hbm, wv_hbm, woT_hbm, w1_hbm, w3_hbm, w2T_hbm,
            outT_hbm,
            qkv_stage, wqkv, woT, w1, w3, w2T, xT, xs, outs,
            h_att, h_ffn, o_scr, act, res_ffn, res_att, edge, att_out, pending, fill_scr, sems,
            *, seg, n_mem):
    seq, d_model = xs.shape
    n_heads, _, d_head = woT.shape
    n_ff = w1.shape[0]
    n_dm = h_att.shape[0]
    n_seg = seq // seg
    m2 = 2 * n_mem
    rows = m2 + 2 * seg
    scale = d_head ** -0.5
    d_main = d_model // LANES * LANES

    n_blk = seq // TOK_BLOCK

    def block(b):
        if isinstance(b, int):
            return pl.ds(b * TOK_BLOCK, TOK_BLOCK)
        return pl.ds(pl.multiple_of(b * TOK_BLOCK, TOK_BLOCK), TOK_BLOCK)

    def slab_copies(src, dst, sem):
        words = src.bitcast(U32)
        return [pltpu.make_async_copy(words.at[:, pl.ds(c * LANES, LANES)], dst.at[c], sem)
                for c in range(n_ff)]

    def x_copies(blocks, sem):
        return [pltpu.make_async_copy(xT_hbm.at[:, block(b)], xT.at[b], sem) for b in blocks]

    def out_copies(blocks, sem):
        return [pltpu.make_async_copy(xT.at[b], outT_hbm.at[:, block(b)], sem) for b in blocks]

    x_early = x_copies(range(EARLY_BLOCKS), sems.at[0])
    w_qkv = [[pltpu.make_async_copy(w, qkv_stage.at[i], sems.at[1 + i])]
             for i, w in enumerate((wq_hbm, wk_hbm, wv_hbm))]
    w_out = [pltpu.make_async_copy(woT_hbm.bitcast(U32), woT, sems.at[4])]
    w_gate = slab_copies(w1_hbm, w1, sems.at[5])
    w_up = slab_copies(w3_hbm, w3, sems.at[6])
    w_down = slab_copies(w2T_hbm, w2T, sems.at[7])
    x_late = x_copies(range(EARLY_BLOCKS, n_blk), sems.at[8])

    def start(copies):
        for c in copies:
            c.start()

    def wait(copies):
        for c in copies:
            c.wait()

    start(x_early + w_qkv[0])

    ri = lax.broadcasted_iota(jnp.int32, (rows, rows), 0)
    ci = lax.broadcasted_iota(jnp.int32, (rows, rows), 1)

    def layer_of(i):
        return jnp.where(i < m2, i // n_mem, (i - m2) // seg)

    def pos_of(i):
        return jnp.where(i < m2, i % n_mem, n_mem + (i - m2) % seg)

    visible = (pos_of(ri) < n_mem) | (pos_of(ri) >= pos_of(ci))
    fill_scr[...] = jnp.where(layer_of(ri) == layer_of(ci),
                              jnp.where(visible, 0.0, -1e9), -jnp.inf).astype(F32)

    def transpose_in(b):
        xs[block(b), :] = xT[b].astype(F32).T.astype(BF16)

    def transpose_out(b):
        xT[b] = outs[block(b), :].astype(F32).T.astype(BF16)

    wait(x_early)
    start(w_qkv[1])
    for b in range(EARLY_BLOCKS):
        transpose_in(b)
    mem0 = mem0_ref[...].astype(F32)
    _store_slabs(h_att, 0, jnp.concatenate([mem0, mem0], axis=0))
    _store_slabs(h_att, m2, _layernorm(xs[0:seg, :].astype(F32)))

    for i in range(3):
        wait(w_qkv[i])
        start((w_qkv[2], w_out, w_gate)[i])

        def regroup(blk, carry, i=i):
            src = pl.ds(pl.multiple_of(blk * (16 * n_heads), 16 * n_heads), 16 * n_heads)
            u = pltpu.bitcast(qkv_stage[i, src, :], U32).reshape(8, 2, n_heads // 2, d_head)
            even = jnp.swapaxes(u[:, 0], 0, 1)
            odd = jnp.swapaxes(u[:, 1], 0, 1)
            lo = (even & jnp.uint32(0xFFFF)) | (odd << 16)
            hi = (even >> 16) | (odd & jnp.uint32(0xFFFF0000))
            dst = pl.ds(pl.multiple_of(blk * 8, 8), 8)
            for h in range(n_heads):
                wqkv[3 * h + i, dst, :] = (lo, hi)[h % 2][h // 2]
            return carry

        lax.fori_loop(0, d_model // 16, regroup, 0)

    def seg_rows(s):
        return pl.ds(s * seg if isinstance(s, int) else pl.multiple_of(s * seg, seg), seg)

    def x_seg(s):
        return xs[seg_rows(s), :].astype(F32)

    def project(hd, n):
        h = _load_slabs(h_att, 0, n_dm, n, d_model)
        qkv = jnp.dot(h, _load_slabs(wqkv, 3 * hd, 3), preferred_element_type=F32).astype(BF16)
        return tuple(qkv[:, i * d_head:(i + 1) * d_head] for i in range(3))

    def scores(q, k):
        n = q.shape[0]
        s = lax.dot_general(q, k, NT_DIMS, preferred_element_type=F32)
        fill = fill_scr[0:n, 0:n]
        s = jnp.where(fill == 0.0, s * scale, fill)
        e = jnp.exp(s - jnp.max(s, axis=-1, keepdims=True))
        total = jnp.sum(e, axis=-1, keepdims=True)
        inv = pl.reciprocal(total, approx=True)
        inv = inv * (2.0 - total * inv)
        return (e * inv).astype(BF16)

    def ffn_up(c, n, slab0=0):
        h = _load_slabs(h_ffn, 0, n_dm, n, d_model)
        w = jnp.concatenate([_load_slabs(w1, c, 1), _load_slabs(w3, c, 1)], axis=1)
        gate_up = jnp.dot(h, w, preferred_element_type=F32)
        half = 0.5 * gate_up[:, :LANES]
        act[slab0 + c, 0:n // 2, :] = _pack((half * jnp.tanh(half) + half) * gate_up[:, LANES:])

    def contract(lhs, rhs, first, count, n, n_out=None, lhs_offset=0):
        return lax.dot_general(_load_slabs(lhs, lhs_offset + first, count, n),
                               _load_slabs(rhs, first, count, n_out),
                               NT_DIMS, preferred_element_type=F32)

    def contract_rest(x, rhs, first, count):
        return lax.dot_general(_load_slabs(rhs, first, count, d_model - d_main, row0=d_main), x,
                               NT_DIMS, preferred_element_type=F32)

    def mix(n_att, n_ffn, act_slab0=0, split=False, before_proj=None):
        qk_delay, pv_delay, n_chunks, spacing = PLAN_WITH_FFN if n_ffn else PLAN_ALONE
        qkv, probs = {}, {}

        def attention_slot(i):
            if 0 <= i - qk_delay < n_heads:
                q, k, _ = qkv[i - qk_delay]
                probs[i - qk_delay] = scores(q, k)
            if 0 <= i - pv_delay < n_heads:
                hd = i - pv_delay
                o = jnp.dot(probs.pop(hd), qkv.pop(hd)[2], preferred_element_type=F32)
                o_scr[hd, 0:n_att // 2, :] = _pack(o)

        ff_done = 0
        for i in range(n_heads):
            qkv[i] = project(i, n_att)
            while n_ffn and ff_done < (i + 1) * n_ff // n_heads:
                ffn_up(ff_done, n_ffn, act_slab0)
                ff_done += 1
            attention_slot(i)
        if before_proj is not None:
            before_proj()
        per = n_heads // n_chunks
        assert pv_delay * spacing * per <= n_heads - pv_delay
        a = rest = None
        for c in range(n_chunks):
            part = contract(o_scr, woT, c * per, per, n_att, d_main if split else None)
            a = part if a is None else a + part
            if split:
                part = contract_rest(_load_slabs(o_scr, c * per, per, n_att), woT, c * per, per)
                rest = part if rest is None else rest + part
            if (c + 1) % spacing == 0:
                attention_slot(n_heads + c // spacing)
        return jnp.concatenate([a, rest.T], axis=1) if split else a

    def ffn_down(n):
        return res_ffn[0:n, :] + contract(act, w2T, 0, n_ff, n)

    def queue_ffn(slot, x):
        res_ffn[seg_rows(slot), :] = x
        _store_slabs(h_ffn, slot * seg, _layernorm(x))

    def set_memory(first, second):
        _store_slabs(h_att, 0, jnp.concatenate([first, second], axis=0))

    one = m2 + seg

    n_pass = 2 * seg
    half_ff = n_ff // 2
    segs_per_blk = TOK_BLOCK // seg
    done_blk = (n_seg - 1 - LAG) // segs_per_blk
    out_early = out_copies(range(done_blk), sems.at[0])
    out_late = out_copies(range(done_blk, n_blk), sems.at[1])

    def advance(t, a, x2):
        x1 = x_seg(t) + a[m2:one]
        x3 = res_att[...] + a[one:]
        set_memory(a[0:n_mem], a[n_mem:m2])
        _store_slabs(h_att, m2, _layernorm(x_seg(jnp.minimum(t + 1, n_seg - 1))))
        res_att[...] = x2
        _store_slabs(h_att, one, _layernorm(x2))
        return x1, x3

    def completed(rest):
        return jnp.concatenate([pending[:, 0:d_main], pending[:, d_main:] + rest], axis=1)

    def steady_step(t, carry):
        pl.when(t == LAG + 1)(lambda: wait(x_late))
        odd = t % 2
        a = mix(rows, n_pass, act_slab0=odd * n_ff, split=True)
        both = jnp.concatenate([_load_slabs(act, j * n_ff + odd * half_ff, half_ff, n_pass)
                                for j in range(2)], axis=0)
        rest = contract_rest(both, w2T, odd * half_ff, half_ff).T
        rest_now = jnp.where(odd == 1, rest[n_pass:], rest[:n_pass])
        y = completed(jnp.where(odd == 1, rest[:n_pass], rest[n_pass:]))
        outs[seg_rows(jnp.maximum(t - 2 - LAG, 0)), :] = y[seg:].astype(BF16)
        x1, x3 = advance(t, a, y[:seg])
        pending[:, 0:d_main] = (res_ffn[0:n_pass, 0:d_main]
                                + contract(act, w2T, 0, n_ff, n_pass, d_main, odd * n_ff))
        pending[:, d_main:] = res_ffn[0:n_pass, d_main:] + rest_now
        queue_ffn(0, x1)
        queue_ffn(1, x3)
        transpose_in(jnp.clip(t - LAG + EARLY_BLOCKS - 1, 0, n_blk - 1))
        transpose_out(jnp.maximum((t - 1 - LAG) // segs_per_blk - 1, 0))
        return carry

    def both_layers():
        x2 = pending[0:seg, :]
        res_att[...] = x2
        _store_slabs(h_att, one, _layernorm(x2))
        pending[0:seg, :] = pending[seg:, :]
        for c in range(n_ff):
            act[(1 - LAG % 2) * n_ff + c] = jnp.zeros(act.shape[1:], U32)
        lax.fori_loop(LAG, n_seg, steady_step, 0)

        odd = n_seg % 2
        last_act = _load_slabs(act, (1 - odd) * n_ff + odd * half_ff, half_ff, n_pass)
        y = completed(contract_rest(last_act, w2T, odd * half_ff, half_ff).T)
        outs[seg_rows(n_seg - 2 - LAG), :] = y[seg:].astype(BF16)
        for b in range((n_seg - 2 - LAG) // segs_per_blk, done_blk):
            transpose_out(b)
        start(out_early)
        edge[seg_rows(LAG + 1), :] = res_att[...]
        edge[seg_rows(LAG + 2), :] = y[:seg]
        mem = _load_slabs(h_att, 0, n_dm, m2, d_model).astype(F32)[n_mem:m2]
        set_memory(mem, mem)
        _store_slabs(h_att, m2, _layernorm(res_att[...]))

    def edge_step(e, carry):
        cur = jnp.where(e < LAG, e, e + 1)
        pl.when(e == LAG - 1)(lambda: start(w_down))

        def before_proj():
            @pl.when(e == 0)
            def _():
                wait(w_out)
                start(w_up)

        a = mix(one, 0, before_proj=before_proj)
        att_out[...] = edge[seg_rows(cur), :] + a[m2:]
        set_memory(a[0:n_mem], mem0_ref[...].astype(F32))

        @pl.when((e == LAG - 1) | (e == LAG))
        def _():
            pl.when(e == LAG - 1)(lambda: wait(w_gate + w_up))
            for c in range(n_ff):
                ffn_up(c, n_pass)

            @pl.when(e == LAG - 1)
            def _():
                wait(w_down)
                start(x_late)

            pending[...] = ffn_down(n_pass)

        @pl.when(e == LAG)
        def _():
            edge[seg_rows(2 * LAG), :] = pending[0:seg, :]
            outs[seg_rows(n_seg - 1 - LAG), :] = pending[seg:, :].astype(BF16)

        _store_slabs(h_att, m2, _layernorm(edge[seg_rows(cur + 1), :]))
        queue_ffn(jnp.where(e < LAG, e % 2, e - LAG), att_out[...])
        pl.when(e == LAG - 1)(both_layers)
        return carry

    n_fill = (LAG + 1) * seg
    edge[0:n_fill, :] = xs[0:n_fill, :].astype(F32)
    edge[n_fill:, :] = jnp.zeros((n_fill, d_model), F32)
    outs[block(0), :] = jnp.zeros((TOK_BLOCK, d_model), BF16)
    lax.fori_loop(0, 2 * LAG, edge_step, 0)

    for c in range(n_ff):
        ffn_up(c, LAG * seg)
    outs[(n_seg - LAG) * seg:, :] = ffn_down(LAG * seg).astype(BF16)
    for b in range(done_blk, n_blk):
        transpose_out(b)
    start(out_late)
    wait(out_early + out_late)


@functools.partial(jax.jit, static_argnames=("A_seg_len",))
def pallas_interleave_layers__memory_aug_recurrent_mem_tr__glu_gated_swiglu__prompt_kernel(
    A_x: jax.Array,
    A_mem0: jax.Array,
    A_Wq: jax.Array,
    A_Wk: jax.Array,
    A_Wv: jax.Array,
    A_Wo: jax.Array,
    A_seg_len: int,
    B_x: jax.Array,
    B_w1: jax.Array,
    B_w3: jax.Array,
    B_w2: jax.Array,
):
    del B_x
    batch, seq, d_model = A_x.shape
    _, n_heads, d_head = A_Wq.shape
    n_mem = A_mem0.shape[1]
    d_ff = B_w1.shape[1]
    seg = int(A_seg_len)
    assert batch == 1 and seq % seg == 0 and seq % TOK_BLOCK == 0
    assert d_head == LANES and d_ff % (2 * LANES) == 0
    rows = 2 * (n_mem + seg)
    n_ff = d_ff // LANES
    n_dm = pl.cdiv(d_model, LANES)

    hbm = pl.BlockSpec(memory_space=pl.ANY)
    outT = pl.pallas_call(
        functools.partial(_kernel, seg=seg, n_mem=n_mem),
        out_shape=jax.ShapeDtypeStruct((d_model, seq), A_x.dtype),
        in_specs=[hbm, pl.BlockSpec(memory_space=pltpu.VMEM)] + [hbm] * 7,
        out_specs=hbm,
        scratch_shapes=[
            pltpu.VMEM((3, d_model * n_heads, d_head), BF16),
            pltpu.VMEM((3 * n_heads, d_model // 2, d_head), U32),
            pltpu.VMEM((n_heads, d_model // 2, d_head), U32),
            pltpu.VMEM((n_ff, d_model // 2, LANES), U32),
            pltpu.VMEM((n_ff, d_model // 2, LANES), U32),
            pltpu.VMEM((n_ff, d_model // 2, LANES), U32),
            pltpu.VMEM((seq // TOK_BLOCK, d_model, TOK_BLOCK), BF16),
            pltpu.VMEM((seq, d_model), BF16),
            pltpu.VMEM((seq, d_model), BF16),
            pltpu.VMEM((n_dm, rows // 2, LANES), U32),
            pltpu.VMEM((n_dm, LAG * seg // 2, LANES), U32),
            pltpu.VMEM((n_heads, rows // 2, d_head), U32),
            pltpu.VMEM((2 * n_ff, LAG * seg // 2, LANES), U32),
            pltpu.VMEM((LAG * seg, d_model), F32),
            pltpu.VMEM((seg, d_model), F32),
            pltpu.VMEM((2 * (LAG + 1) * seg, d_model), F32),
            pltpu.VMEM((seg, d_model), F32),
            pltpu.VMEM((2 * seg, d_model), F32),
            pltpu.VMEM((rows, rows), F32),
            pltpu.SemaphoreType.DMA((9,)),
        ],
        compiler_params=pltpu.CompilerParams(vmem_limit_bytes=100 * 1024 * 1024),
    )(
        A_x[0].T,
        A_mem0[0],
        A_Wq.reshape(d_model * n_heads, d_head),
        A_Wk.reshape(d_model * n_heads, d_head),
        A_Wv.reshape(d_model * n_heads, d_head),
        jnp.transpose(A_Wo, (0, 2, 1)),
        B_w1,
        B_w3,
        B_w2.T,
    )
    return outT.T[None]
```

```python
import functools

import jax
import jax.numpy as jnp
from jax import lax
import jax.experimental.pallas as pl
import jax.experimental.pallas.tpu as pltpu

F32 = jnp.float32
BF16 = jnp.bfloat16
U32 = jnp.uint32
LANES = 128
LAG = 3
PLAN_WITH_FFN = (1, 3, 8, 2)
PLAN_ALONE = (2, 5, 16, 2)
TOK_BLOCK = 128
EARLY_BLOCKS = 2
DOWN_CHUNKS = 2
NT_DIMS = (((1,), (1,)), ((), ()))


def _layernorm(x):
    mean = jnp.mean(x, axis=-1, keepdims=True)
    xc = x - mean
    var = jnp.mean(xc * xc, axis=-1, keepdims=True)
    return xc * lax.rsqrt(var + 1e-5)


def _pack(x):
    return pltpu.bitcast(x.astype(BF16), U32)


def _rows(start, size):
    return pl.ds(start if isinstance(start, int) else pl.multiple_of(start, 8), size)


def _load_slabs(ref, first, count, n_rows=None, width=None, row0=0):
    words = slice(row0 // 2, ref.shape[1] if n_rows is None else (row0 + n_rows) // 2)
    lanes = [LANES] * count
    if width is not None and width % LANES:
        lanes[-1] = width % LANES
    parts = [pltpu.bitcast(ref[first + i, words, 0:lanes[i]], BF16) for i in range(count)]
    return parts[0] if count == 1 else jnp.concatenate(parts, axis=1)


def _store_slabs(ref, row0, value):
    words = _pack(value)
    n_rows, width = words.shape
    for i in range(pl.cdiv(width, LANES)):
        part = words[:, i * LANES:min(width, (i + 1) * LANES)]
        ref[i, _rows(row0 // 2, n_rows), 0:part.shape[1]] = part


def _kernel(xT_hbm, mem0_ref, wq_hbm, wk_hbm, wv_hbm, woT_hbm, w1_hbm, w3_hbm, w2T_hbm,
            outT_hbm,
            qkv_stage, wqkv, woT, w1, w3, w2T, xT, xs, outs,
            h_att, h_ffn, o_scr, act, res_ffn, res_att, edge, att_out, pending, fill_scr, sems,
            *, seg, n_mem):
    seq, d_model = xs.shape
    n_heads, _, d_head = woT.shape
    n_ff = w1.shape[0]
    n_dm = h_att.shape[0]
    n_seg = seq // seg
    m2 = 2 * n_mem
    rows = m2 + 2 * seg
    scale = d_head ** -0.5
    d_main = d_model // LANES * LANES

    n_blk = seq // TOK_BLOCK

    def block(b):
        if isinstance(b, int):
            return pl.ds(b * TOK_BLOCK, TOK_BLOCK)
        return pl.ds(pl.multiple_of(b * TOK_BLOCK, TOK_BLOCK), TOK_BLOCK)

    def slab_copies(src, dst, sem, slabs):
        words = src.bitcast(U32)
        return [pltpu.make_async_copy(words.at[:, pl.ds(c * LANES, LANES)], dst.at[c], sem)
                for c in slabs]

    def x_copies(blocks, sem):
        return [pltpu.make_async_copy(xT_hbm.at[:, block(b)], xT.at[b], sem) for b in blocks]

    def out_copies(blocks, sem):
        return [pltpu.make_async_copy(xT.at[b], outT_hbm.at[:, block(b)], sem) for b in blocks]

    x_early = x_copies(range(EARLY_BLOCKS), sems.at[0])
    w_qkv = [[pltpu.make_async_copy(w, qkv_stage.at[i], sems.at[1 + i])]
             for i, w in enumerate((wq_hbm, wk_hbm, wv_hbm))]
    w_out = [pltpu.make_async_copy(woT_hbm.bitcast(U32), woT, sems.at[4])]
    w_gate = slab_copies(w1_hbm, w1, sems.at[5], range(n_ff))
    w_up = slab_copies(w3_hbm, w3, sems.at[6], range(n_ff))
    down_slabs = n_ff // DOWN_CHUNKS
    w_down = [slab_copies(w2T_hbm, w2T, sems.at[8 + i], range(i * down_slabs, (i + 1) * down_slabs))
              for i in range(DOWN_CHUNKS)]
    x_late = x_copies(range(EARLY_BLOCKS, n_blk), sems.at[7])

    def start(copies):
        for c in copies:
            c.start()

    def wait(copies):
        for c in copies:
            c.wait()

    start(x_early + w_qkv[0])

    ri = lax.broadcasted_iota(jnp.int32, (rows, rows), 0)
    ci = lax.broadcasted_iota(jnp.int32, (rows, rows), 1)

    def layer_of(i):
        return jnp.where(i < m2, i // n_mem, (i - m2) // seg)

    def pos_of(i):
        return jnp.where(i < m2, i % n_mem, n_mem + (i - m2) % seg)

    visible = (pos_of(ri) < n_mem) | (pos_of(ri) >= pos_of(ci))
    fill_scr[...] = jnp.where(layer_of(ri) == layer_of(ci),
                              jnp.where(visible, 0.0, -1e9), -jnp.inf).astype(F32)

    def transpose_in(b):
        xs[block(b), :] = xT[b].astype(F32).T.astype(BF16)

    def transpose_out(b):
        xT[b] = outs[block(b), :].astype(F32).T.astype(BF16)

    wait(x_early)
    start(w_qkv[1])
    for b in range(EARLY_BLOCKS):
        transpose_in(b)
    mem0 = mem0_ref[...].astype(F32)
    _store_slabs(h_att, 0, jnp.concatenate([mem0, mem0], axis=0))
    _store_slabs(h_att, m2, _layernorm(xs[0:seg, :].astype(F32)))

    for i in range(3):
        wait(w_qkv[i])
        start((w_qkv[2], w_out, w_gate)[i])

        def regroup(blk, carry, i=i):
            src = pl.ds(pl.multiple_of(blk * (16 * n_heads), 16 * n_heads), 16 * n_heads)
            u = pltpu.bitcast(qkv_stage[i, src, :], U32).reshape(8, 2, n_heads // 2, d_head)
            even = jnp.swapaxes(u[:, 0], 0, 1)
            odd = jnp.swapaxes(u[:, 1], 0, 1)
            lo = (even & jnp.uint32(0xFFFF)) | (odd << 16)
            hi = (even >> 16) | (odd & jnp.uint32(0xFFFF0000))
            dst = pl.ds(pl.multiple_of(blk * 8, 8), 8)
            for h in range(n_heads):
                wqkv[3 * h + i, dst, :] = (lo, hi)[h % 2][h // 2]
            return carry

        lax.fori_loop(0, d_model // 16, regroup, 0)

    def seg_rows(s):
        return pl.ds(s * seg if isinstance(s, int) else pl.multiple_of(s * seg, seg), seg)

    def x_seg(s):
        return xs[seg_rows(s), :].astype(F32)

    def project(hd, n):
        h = _load_slabs(h_att, 0, n_dm, n, d_model)
        qkv = jnp.dot(h, _load_slabs(wqkv, 3 * hd, 3), preferred_element_type=F32).astype(BF16)
        return tuple(qkv[:, i * d_head:(i + 1) * d_head] for i in range(3))

    def scores(q, k):
        n = q.shape[0]
        s = lax.dot_general(q, k, NT_DIMS, preferred_element_type=F32)
        fill = fill_scr[0:n, 0:n]
        s = jnp.where(fill == 0.0, s * scale, fill)
        e = jnp.exp(s - jnp.max(s, axis=-1, keepdims=True))
        total = jnp.sum(e, axis=-1, keepdims=True)
        inv = pl.reciprocal(total, approx=True)
        inv = inv * (2.0 - total * inv)
        return (e * inv).astype(BF16)

    def ffn_up(c, n, slab0=0):
        h = _load_slabs(h_ffn, 0, n_dm, n, d_model)
        w = jnp.concatenate([_load_slabs(w1, c, 1), _load_slabs(w3, c, 1)], axis=1)
        gate_up = jnp.dot(h, w, preferred_element_type=F32)
        half = 0.5 * gate_up[:, :LANES]
        act[slab0 + c, 0:n // 2, :] = _pack((half * jnp.tanh(half) + half) * gate_up[:, LANES:])

    def contract(lhs, rhs, first, count, n, n_out=None, lhs_offset=0):
        return lax.dot_general(_load_slabs(lhs, lhs_offset + first, count, n),
                               _load_slabs(rhs, first, count, n_out),
                               NT_DIMS, preferred_element_type=F32)

    def contract_rest(x, rhs, first, count):
        return lax.dot_general(_load_slabs(rhs, first, count, d_model - d_main, row0=d_main), x,
                               NT_DIMS, preferred_element_type=F32)

    def mix(n_att, n_ffn, act_slab0=0, split=False, before_proj=None):
        qk_delay, pv_delay, n_chunks, spacing = PLAN_WITH_FFN if n_ffn else PLAN_ALONE
        qkv, probs = {}, {}

        def attention_slot(i):
            if 0 <= i - qk_delay < n_heads:
                q, k, _ = qkv[i - qk_delay]
                probs[i - qk_delay] = scores(q, k)
            if 0 <= i - pv_delay < n_heads:
                hd = i - pv_delay
                o = jnp.dot(probs.pop(hd), qkv.pop(hd)[2], preferred_element_type=F32)
                o_scr[hd, 0:n_att // 2, :] = _pack(o)

        ff_done = 0
        for i in range(n_heads):
            qkv[i] = project(i, n_att)
            while n_ffn and ff_done < (i + 1) * n_ff // n_heads:
                ffn_up(ff_done, n_ffn, act_slab0)
                ff_done += 1
            attention_slot(i)
        if before_proj is not None:
            before_proj()
        per = n_heads // n_chunks
        assert pv_delay * spacing * per <= n_heads - pv_delay
        a = rest = None
        for c in range(n_chunks):
            part = contract(o_scr, woT, c * per, per, n_att, d_main if split else None)
            a = part if a is None else a + part
            if split:
                part = contract_rest(_load_slabs(o_scr, c * per, per, n_att), woT, c * per, per)
                rest = part if rest is None else rest + part
            if (c + 1) % spacing == 0:
                attention_slot(n_heads + c // spacing)
        return jnp.concatenate([a, rest.T], axis=1) if split else a

    def queue_ffn(slot, x):
        res_ffn[seg_rows(slot), :] = x
        _store_slabs(h_ffn, slot * seg, _layernorm(x))

    def set_memory(first, second):
        _store_slabs(h_att, 0, jnp.concatenate([first, second], axis=0))

    one = m2 + seg
    n_pass = 2 * seg
    half_ff = n_ff // 2
    segs_per_blk = TOK_BLOCK // seg
    done_blk = (n_seg - 1 - LAG) // segs_per_blk
    out_early = out_copies(range(done_blk), sems.at[0])
    out_late = out_copies(range(done_blk, n_blk), sems.at[1])

    def advance(t, a, x2):
        x1 = x_seg(t) + a[m2:one]
        x3 = res_att[...] + a[one:]
        set_memory(a[0:n_mem], a[n_mem:m2])
        _store_slabs(h_att, m2, _layernorm(x_seg(jnp.minimum(t + 1, n_seg - 1))))
        res_att[...] = x2
        _store_slabs(h_att, one, _layernorm(x2))
        return x1, x3

    def completed(rest):
        return jnp.concatenate([pending[:, 0:d_main], pending[:, d_main:] + rest], axis=1)

    def steady_step(t, carry):
        pl.when(t == LAG + 1)(lambda: wait(x_late))
        transpose_in(jnp.clip(t - LAG + EARLY_BLOCKS - 1, 0, n_blk - 1))
        transpose_out(jnp.maximum((t - 2 - LAG) // segs_per_blk - 1, 0))
        odd = t % 2
        a = mix(rows, n_pass, act_slab0=odd * n_ff, split=True)
        both = jnp.concatenate([_load_slabs(act, j * n_ff + odd * half_ff, half_ff, n_pass)
                                for j in range(2)], axis=0)
        rest = contract_rest(both, w2T, odd * half_ff, half_ff).T
        rest_now = jnp.where(odd == 1, rest[n_pass:], rest[:n_pass])
        y = completed(jnp.where(odd == 1, rest[:n_pass], rest[n_pass:]))
        outs[seg_rows(jnp.maximum(t - 2 - LAG, 0)), :] = y[seg:].astype(BF16)
        x1, x3 = advance(t, a, y[:seg])
        pending[:, 0:d_main] = (res_ffn[0:n_pass, 0:d_main]
                                + contract(act, w2T, 0, n_ff, n_pass, d_main, odd * n_ff))
        pending[:, d_main:] = res_ffn[0:n_pass, d_main:] + rest_now
        queue_ffn(0, x1)
        queue_ffn(1, x3)
        return carry

    def both_layers():
        start(x_late)
        x2 = pending[0:seg, :]
        res_att[...] = x2
        _store_slabs(h_att, one, _layernorm(x2))
        pending[0:seg, :] = pending[seg:, :]
        for c in range(n_ff):
            act[(1 - LAG % 2) * n_ff + c] = jnp.zeros(act.shape[1:], U32)
        lax.fori_loop(LAG, n_seg, steady_step, 0)

        odd = n_seg % 2
        last_act = _load_slabs(act, (1 - odd) * n_ff + odd * half_ff, half_ff, n_pass)
        y = completed(contract_rest(last_act, w2T, odd * half_ff, half_ff).T)
        outs[seg_rows(n_seg - 2 - LAG), :] = y[seg:].astype(BF16)
        for b in range((n_seg - 3 - LAG) // segs_per_blk, done_blk):
            transpose_out(b)
        start(out_early)
        edge[seg_rows(LAG + 1), :] = res_att[...]
        edge[seg_rows(LAG + 2), :] = y[:seg]
        mem = _load_slabs(h_att, 0, n_dm, m2, d_model).astype(F32)[n_mem:m2]
        set_memory(mem, mem)
        _store_slabs(h_att, m2, _layernorm(res_att[...]))

    def edge_step(e, carry):
        cur = jnp.where(e < LAG, e, e + 1)
        pl.when(e == LAG - 1)(lambda: start(sum(w_down, [])))

        def before_proj():
            @pl.when(e == 0)
            def _():
                wait(w_out)
                start(w_up)

        a = mix(one, 0, before_proj=before_proj)
        att_out[...] = edge[seg_rows(cur), :] + a[m2:]
        set_memory(a[0:n_mem], mem0_ref[...].astype(F32))

        @pl.when((e == LAG - 1) | (e == LAG))
        def _():
            pl.when(e == LAG - 1)(lambda: wait(w_gate + w_up))
            for c in range(n_ff):
                ffn_up(c, n_pass)
            pending[...] = res_ffn[0:n_pass, :]
            for i in range(DOWN_CHUNKS):
                pl.when(e == LAG - 1)(functools.partial(wait, w_down[i]))
                pending[...] += contract(act, w2T, i * down_slabs, down_slabs, n_pass)

        @pl.when(e == LAG)
        def _():
            edge[seg_rows(2 * LAG), :] = pending[0:seg, :]
            outs[seg_rows(n_seg - 1 - LAG), :] = pending[seg:, :].astype(BF16)

        _store_slabs(h_att, m2, _layernorm(edge[seg_rows(cur + 1), :]))
        queue_ffn(jnp.where(e < LAG, e % 2, e - LAG), att_out[...])
        pl.when(e == LAG - 1)(both_layers)
        return carry

    n_fill = (LAG + 1) * seg
    edge[0:n_fill, :] = xs[0:n_fill, :].astype(F32)
    edge[n_fill:, :] = jnp.zeros((n_fill, d_model), F32)
    outs[block(0), :] = jnp.zeros((TOK_BLOCK, d_model), BF16)
    lax.fori_loop(0, 2 * LAG, edge_step, 0)

    for c in range(n_ff):
        ffn_up(c, LAG * seg)
    y = jnp.concatenate([contract(act, w2T, 0, n_ff, LAG * seg, d_main),
                         contract_rest(_load_slabs(act, 0, n_ff, LAG * seg), w2T, 0, n_ff).T], axis=1)
    outs[(n_seg - LAG) * seg:, :] = (res_ffn[...] + y).astype(BF16)
    for b in range(done_blk, n_blk):
        transpose_out(b)
    start(out_late)
    wait(out_early + out_late)


@functools.partial(jax.jit, static_argnames=("A_seg_len",))
def pallas_interleave_layers__memory_aug_recurrent_mem_tr__glu_gated_swiglu__prompt_kernel(
    A_x: jax.Array,
    A_mem0: jax.Array,
    A_Wq: jax.Array,
    A_Wk: jax.Array,
    A_Wv: jax.Array,
    A_Wo: jax.Array,
    A_seg_len: int,
    B_x: jax.Array,
    B_w1: jax.Array,
    B_w3: jax.Array,
    B_w2: jax.Array,
):
    del B_x
    batch, seq, d_model = A_x.shape
    _, n_heads, d_head = A_Wq.shape
    n_mem = A_mem0.shape[1]
    d_ff = B_w1.shape[1]
    seg = int(A_seg_len)
    assert batch == 1 and seq % seg == 0 and seq % TOK_BLOCK == 0
    assert d_head == LANES and d_ff % (2 * DOWN_CHUNKS * LANES) == 0
    assert TOK_BLOCK == (LAG + 1) * seg and seg % 16 == 0 and n_mem % 8 == 0
    assert d_model % 16 == 0 and d_model % LANES != 0 and n_heads % 16 == 0
    rows = 2 * (n_mem + seg)
    n_ff = d_ff // LANES
    n_dm = pl.cdiv(d_model, LANES)

    hbm = pl.BlockSpec(memory_space=pl.ANY)
    outT = pl.pallas_call(
        functools.partial(_kernel, seg=seg, n_mem=n_mem),
        out_shape=jax.ShapeDtypeStruct((d_model, seq), A_x.dtype),
        in_specs=[hbm, pl.BlockSpec(memory_space=pltpu.VMEM)] + [hbm] * 7,
        out_specs=hbm,
        scratch_shapes=[
            pltpu.VMEM((3, d_model * n_heads, d_head), BF16),
            pltpu.VMEM((3 * n_heads, d_model // 2, d_head), U32),
            pltpu.VMEM((n_heads, d_model // 2, d_head), U32),
            pltpu.VMEM((n_ff, d_model // 2, LANES), U32),
            pltpu.VMEM((n_ff, d_model // 2, LANES), U32),
            pltpu.VMEM((n_ff, d_model // 2, LANES), U32),
            pltpu.VMEM((seq // TOK_BLOCK, d_model, TOK_BLOCK), BF16),
            pltpu.VMEM((seq, d_model), BF16),
            pltpu.VMEM((seq, d_model), BF16),
            pltpu.VMEM((n_dm, rows // 2, LANES), U32),
            pltpu.VMEM((n_dm, LAG * seg // 2, LANES), U32),
            pltpu.VMEM((n_heads, rows // 2, d_head), U32),
            pltpu.VMEM((2 * n_ff, LAG * seg // 2, LANES), U32),
            pltpu.VMEM((LAG * seg, d_model), F32),
            pltpu.VMEM((seg, d_model), F32),
            pltpu.VMEM((2 * (LAG + 1) * seg, d_model), F32),
            pltpu.VMEM((seg, d_model), F32),
            pltpu.VMEM((2 * seg, d_model), F32),
            pltpu.VMEM((rows, rows), F32),
            pltpu.SemaphoreType.DMA((8 + DOWN_CHUNKS,)),
        ],
        compiler_params=pltpu.CompilerParams(vmem_limit_bytes=100 * 1024 * 1024),
    )(
        A_x[0].T,
        A_mem0[0],
        A_Wq.reshape(d_model * n_heads, d_head),
        A_Wk.reshape(d_model * n_heads, d_head),
        A_Wv.reshape(d_model * n_heads, d_head),
        jnp.transpose(A_Wo, (0, 2, 1)),
        B_w1,
        B_w3,
        B_w2.T,
    )
    return outT.T[None]
```

```python
import functools

import jax
import jax.numpy as jnp
from jax import lax
import jax.experimental.pallas as pl
import jax.experimental.pallas.tpu as pltpu

F32 = jnp.float32
BF16 = jnp.bfloat16
U32 = jnp.uint32
LANES = 128
LAG = 3
PLAN_WITH_FFN = (1, 3, 8, 2)
PLAN_ALONE = (2, 5, 16, 2)
TOK_BLOCK = 128
EARLY_BLOCKS = 2
NT_DIMS = (((1,), (1,)), ((), ()))


def _layernorm(x):
    mean = jnp.mean(x, axis=-1, keepdims=True)
    xc = x - mean
    var = jnp.mean(xc * xc, axis=-1, keepdims=True)
    return xc * lax.rsqrt(var + 1e-5)


def _pack(x):
    return pltpu.bitcast(x.astype(BF16), U32)


def _rows(start, size):
    return pl.ds(start if isinstance(start, int) else pl.multiple_of(start, 8), size)


def _load_slabs(ref, first, count, n_rows=None, width=None, row0=0):
    words = slice(row0 // 2, ref.shape[1] if n_rows is None else (row0 + n_rows) // 2)
    lanes = [LANES] * count
    if width is not None and width % LANES:
        lanes[-1] = width % LANES
    parts = [pltpu.bitcast(ref[first + i, words, 0:lanes[i]], BF16) for i in range(count)]
    return parts[0] if count == 1 else jnp.concatenate(parts, axis=1)


def _store_slabs(ref, row0, value):
    words = _pack(value)
    n_rows, width = words.shape
    for i in range(pl.cdiv(width, LANES)):
        part = words[:, i * LANES:min(width, (i + 1) * LANES)]
        ref[i, _rows(row0 // 2, n_rows), 0:part.shape[1]] = part


def _kernel(xT_hbm, mem0_ref, wq_hbm, wk_hbm, wv_hbm, woT_hbm, w1_hbm, w3_hbm, w2T_hbm,
            outT_hbm,
            qkv_stage, wo_stage, ff_stage, wqkv, woT, w1, w3, w2T, xT, xs, outs,
            h_att, h_ffn, o_scr, act, res_ffn, res_att, edge, att_out, pending, fill_scr, sems, qkv_sems,
            *, seg, n_mem):
    seq, d_model = xs.shape
    n_heads, _, d_head = woT.shape
    n_ff = w1.shape[0]
    n_dm = h_att.shape[0]
    n_seg = seq // seg
    m2 = 2 * n_mem
    rows = m2 + 2 * seg
    scale = d_head ** -0.5
    d_main = d_model // LANES * LANES

    n_blk = seq // TOK_BLOCK

    def block(b):
        if isinstance(b, int):
            return pl.ds(b * TOK_BLOCK, TOK_BLOCK)
        return pl.ds(pl.multiple_of(b * TOK_BLOCK, TOK_BLOCK), TOK_BLOCK)

    def slab_copies(src, which, sem):
        return [pltpu.make_async_copy(src.at[:, pl.ds(c * LANES, LANES)], ff_stage.at[which * n_ff + c], sem)
                for c in range(n_ff)]

    def repack(stage, offset, dst):
        def copy(c, carry):
            dst[c] = pltpu.bitcast(stage[offset + c], U32)
            return carry

        lax.fori_loop(0, dst.shape[0], copy, 0, unroll=4)

    def x_copies(blocks, sem):
        return [pltpu.make_async_copy(xT_hbm.at[:, block(b)], xT.at[b], sem) for b in blocks]

    def out_copies(blocks, sem):
        return [pltpu.make_async_copy(xT.at[b], outT_hbm.at[:, block(b)], sem) for b in blocks]

    x_early = x_copies(range(EARLY_BLOCKS), sems.at[0])
    half_rows = qkv_stage.shape[1] // 2
    w_qkv = [[pltpu.make_async_copy(w.at[pl.ds(j * half_rows, half_rows)],
                                    qkv_stage.at[i, pl.ds(j * half_rows, half_rows)],
                                    qkv_sems.at[2 * i + j]) for j in range(2)]
             for i, w in enumerate((wq_hbm, wk_hbm, wv_hbm))]
    w_out = [pltpu.make_async_copy(woT_hbm, wo_stage, sems.at[4])]
    w_gate = slab_copies(w1_hbm, 0, sems.at[5])
    w_up = slab_copies(w3_hbm, 1, sems.at[6])
    w_down = slab_copies(w2T_hbm, 2, sems.at[8])
    x_late = x_copies(range(EARLY_BLOCKS, n_blk), sems.at[7])

    def start(copies):
        for c in copies:
            c.start()

    def wait(copies):
        for c in copies:
            c.wait()

    start(x_early + w_qkv[0])

    ri = lax.broadcasted_iota(jnp.int32, (rows, rows), 0)
    ci = lax.broadcasted_iota(jnp.int32, (rows, rows), 1)

    def layer_of(i):
        return jnp.where(i < m2, i // n_mem, (i - m2) // seg)

    def pos_of(i):
        return jnp.where(i < m2, i % n_mem, n_mem + (i - m2) % seg)

    visible = (pos_of(ri) < n_mem) | (pos_of(ri) >= pos_of(ci))
    fill_scr[...] = jnp.where(layer_of(ri) == layer_of(ci),
                              jnp.where(visible, 0.0, -1e9), -jnp.inf).astype(F32)

    def transpose_in(b):
        xs[block(b), :] = xT[b].astype(F32).T.astype(BF16)

    def transpose_out(b):
        xT[b] = outs[block(b), :].astype(F32).T.astype(BF16)

    wait(x_early)
    start(w_qkv[1])
    for b in range(EARLY_BLOCKS):
        transpose_in(b)
    mem0 = mem0_ref[...].astype(F32)
    _store_slabs(h_att, 0, jnp.concatenate([mem0, mem0], axis=0))
    _store_slabs(h_att, m2, _layernorm(xs[0:seg, :].astype(F32)))

    for i in range(3):
        def regroup(blk, carry, i=i):
            src = pl.ds(pl.multiple_of(blk * (16 * n_heads), 16 * n_heads), 16 * n_heads)
            u = pltpu.bitcast(qkv_stage[i, src, :], U32).reshape(8, 2, n_heads // 2, d_head)
            even = jnp.swapaxes(u[:, 0], 0, 1)
            odd = jnp.swapaxes(u[:, 1], 0, 1)
            lo = (even & jnp.uint32(0xFFFF)) | (odd << 16)
            hi = (even >> 16) | (odd & jnp.uint32(0xFFFF0000))
            dst = pl.ds(pl.multiple_of(blk * 8, 8), 8)
            for h in range(n_heads):
                wqkv[3 * h + i, dst, :] = (lo, hi)[h % 2][h // 2]
            return carry

        n_half = d_model // 32
        w_qkv[i][0].wait()
        lax.fori_loop(0, n_half, regroup, 0)
        w_qkv[i][1].wait()
        start((w_qkv[2], w_out, w_gate)[i])
        lax.fori_loop(n_half, 2 * n_half, regroup, 0)

    def seg_rows(s):
        return pl.ds(s * seg if isinstance(s, int) else pl.multiple_of(s * seg, seg), seg)

    def x_seg(s):
        return xs[seg_rows(s), :].astype(F32)

    def project(hd, n):
        h = _load_slabs(h_att, 0, n_dm, n, d_model)
        qkv = jnp.dot(h, _load_slabs(wqkv, 3 * hd, 3), preferred_element_type=F32).astype(BF16)
        return tuple(qkv[:, i * d_head:(i + 1) * d_head] for i in range(3))

    def scores(q, k):
        n = q.shape[0]
        s = lax.dot_general(q, k, NT_DIMS, preferred_element_type=F32)
        fill = fill_scr[0:n, 0:n]
        s = jnp.where(fill == 0.0, s * scale, fill)
        e = jnp.exp(s - jnp.max(s, axis=-1, keepdims=True))
        total = jnp.sum(e, axis=-1, keepdims=True)
        inv = pl.reciprocal(total, approx=True)
        inv = inv * (2.0 - total * inv)
        return (e * inv).astype(BF16)

    def ffn_up(c, n, slab0=0):
        h = _load_slabs(h_ffn, 0, n_dm, n, d_model)
        w = jnp.concatenate([_load_slabs(w1, c, 1), _load_slabs(w3, c, 1)], axis=1)
        gate_up = jnp.dot(h, w, preferred_element_type=F32)
        half = 0.5 * gate_up[:, :LANES]
        act[slab0 + c, 0:n // 2, :] = _pack((half * jnp.tanh(half) + half) * gate_up[:, LANES:])

    def contract(lhs, rhs, first, count, n, n_out=None, lhs_offset=0):
        return lax.dot_general(_load_slabs(lhs, lhs_offset + first, count, n),
                               _load_slabs(rhs, first, count, n_out),
                               NT_DIMS, preferred_element_type=F32)

    def contract_rest(x, rhs, first, count):
        return lax.dot_general(_load_slabs(rhs, first, count, d_model - d_main, row0=d_main), x,
                               NT_DIMS, preferred_element_type=F32)

    def mix(n_att, n_ffn, act_slab0=0, split=False, before_proj=None):
        qk_delay, pv_delay, n_chunks, spacing = PLAN_WITH_FFN if n_ffn else PLAN_ALONE
        qkv, probs = {}, {}

        def attention_slot(i):
            if 0 <= i - qk_delay < n_heads:
                q, k, _ = qkv[i - qk_delay]
                probs[i - qk_delay] = scores(q, k)
            if 0 <= i - pv_delay < n_heads:
                hd = i - pv_delay
                o = jnp.dot(probs.pop(hd), qkv.pop(hd)[2], preferred_element_type=F32)
                o_scr[hd, 0:n_att // 2, :] = _pack(o)

        ff_done = 0
        for i in range(n_heads):
            qkv[i] = project(i, n_att)
            while n_ffn and ff_done < (i + 1) * n_ff // n_heads:
                ffn_up(ff_done, n_ffn, act_slab0)
                ff_done += 1
            attention_slot(i)
        if before_proj is not None:
            before_proj()
        per = n_heads // n_chunks
        assert pv_delay * spacing * per <= n_heads - pv_delay
        a = rest = None
        for c in range(n_chunks):
            part = contract(o_scr, woT, c * per, per, n_att, d_main if split else None)
            a = part if a is None else a + part
            if split:
                part = contract_rest(_load_slabs(o_scr, c * per, per, n_att), woT, c * per, per)
                rest = part if rest is None else rest + part
            if (c + 1) % spacing == 0:
                attention_slot(n_heads + c // spacing)
        return jnp.concatenate([a, rest.T], axis=1) if split else a

    def queue_ffn(slot, x):
        res_ffn[seg_rows(slot), :] = x
        _store_slabs(h_ffn, slot * seg, _layernorm(x))

    def set_memory(first, second):
        _store_slabs(h_att, 0, jnp.concatenate([first, second], axis=0))

    one = m2 + seg
    n_pass = 2 * seg
    half_ff = n_ff // 2
    segs_per_blk = TOK_BLOCK // seg
    done_blk = (n_seg - 1 - LAG) // segs_per_blk
    out_early = out_copies(range(done_blk), sems.at[0])
    out_late = out_copies(range(done_blk, n_blk), sems.at[1])

    def advance(t, a, x2):
        x1 = x_seg(t) + a[m2:one]
        x3 = res_att[...] + a[one:]
        set_memory(a[0:n_mem], a[n_mem:m2])
        _store_slabs(h_att, m2, _layernorm(x_seg(jnp.minimum(t + 1, n_seg - 1))))
        res_att[...] = x2
        _store_slabs(h_att, one, _layernorm(x2))
        return x1, x3

    def completed(rest):
        return jnp.concatenate([pending[:, 0:d_main], pending[:, d_main:] + rest], axis=1)

    def steady_step(t, carry):
        pl.when(t == LAG + 1)(lambda: wait(x_late))
        transpose_in(jnp.clip(t - LAG + EARLY_BLOCKS - 1, 0, n_blk - 1))
        transpose_out(jnp.maximum((t - 2 - LAG) // segs_per_blk - 1, 0))
        odd = t % 2
        a = mix(rows, n_pass, act_slab0=odd * n_ff, split=True)
        both = jnp.concatenate([_load_slabs(act, j * n_ff + odd * half_ff, half_ff, n_pass)
                                for j in range(2)], axis=0)
        rest = contract_rest(both, w2T, odd * half_ff, half_ff).T
        rest_now = jnp.where(odd == 1, rest[n_pass:], rest[:n_pass])
        y = completed(jnp.where(odd == 1, rest[:n_pass], rest[n_pass:]))
        outs[seg_rows(jnp.maximum(t - 2 - LAG, 0)), :] = y[seg:].astype(BF16)
        x1, x3 = advance(t, a, y[:seg])
        pending[:, 0:d_main] = (res_ffn[0:n_pass, 0:d_main]
                                + contract(act, w2T, 0, n_ff, n_pass, d_main, odd * n_ff))
        pending[:, d_main:] = res_ffn[0:n_pass, d_main:] + rest_now
        queue_ffn(0, x1)
        queue_ffn(1, x3)
        return carry

    def both_layers():
        start(x_late)
        x2 = pending[0:seg, :]
        res_att[...] = x2
        _store_slabs(h_att, one, _layernorm(x2))
        pending[0:seg, :] = pending[seg:, :]
        for c in range(n_ff):
            act[(1 - LAG % 2) * n_ff + c] = jnp.zeros(act.shape[1:], U32)
        lax.fori_loop(LAG, n_seg, steady_step, 0)

        odd = n_seg % 2
        last_act = _load_slabs(act, (1 - odd) * n_ff + odd * half_ff, half_ff, n_pass)
        y = completed(contract_rest(last_act, w2T, odd * half_ff, half_ff).T)
        outs[seg_rows(n_seg - 2 - LAG), :] = y[seg:].astype(BF16)
        for b in range((n_seg - 3 - LAG) // segs_per_blk, done_blk):
            transpose_out(b)
        start(out_early)
        edge[seg_rows(LAG + 1), :] = res_att[...]
        edge[seg_rows(LAG + 2), :] = y[:seg]
        mem = _load_slabs(h_att, 0, n_dm, m2, d_model).astype(F32)[n_mem:m2]
        set_memory(mem, mem)
        _store_slabs(h_att, m2, _layernorm(res_att[...]))

    def edge_step(e, carry):
        cur = jnp.where(e < LAG, e, e + 1)

        @pl.when(e == LAG - 1)
        def _():
            start(w_down)
            wait(w_gate)
            repack(ff_stage, 0, w1)

        def before_proj():
            @pl.when(e == 0)
            def _():
                wait(w_out)
                start(w_up)
                repack(wo_stage, 0, woT)

        a = mix(one, 0, before_proj=before_proj)
        att_out[...] = edge[seg_rows(cur), :] + a[m2:]
        set_memory(a[0:n_mem], mem0_ref[...].astype(F32))

        @pl.when((e == LAG - 1) | (e == LAG))
        def _():
            @pl.when(e == LAG - 1)
            def _():
                wait(w_up)
                repack(ff_stage, n_ff, w3)
            for c in range(n_ff):
                ffn_up(c, n_pass)

            @pl.when(e == LAG - 1)
            def _():
                wait(w_down)
                repack(ff_stage, 2 * n_ff, w2T)

            pending[...] = res_ffn[0:n_pass, :] + contract(act, w2T, 0, n_ff, n_pass)

        @pl.when(e == LAG)
        def _():
            edge[seg_rows(2 * LAG), :] = pending[0:seg, :]
            outs[seg_rows(n_seg - 1 - LAG), :] = pending[seg:, :].astype(BF16)

        _store_slabs(h_att, m2, _layernorm(edge[seg_rows(cur + 1), :]))
        queue_ffn(jnp.where(e < LAG, e % 2, e - LAG), att_out[...])
        pl.when(e == LAG - 1)(both_layers)
        return carry

    n_fill = (LAG + 1) * seg
    edge[0:n_fill, :] = xs[0:n_fill, :].astype(F32)
    edge[n_fill:, :] = jnp.zeros((n_fill, d_model), F32)
    outs[block(0), :] = jnp.zeros((TOK_BLOCK, d_model), BF16)
    lax.fori_loop(0, 2 * LAG, edge_step, 0)

    for c in range(n_ff):
        ffn_up(c, LAG * seg)
    y = jnp.concatenate([contract(act, w2T, 0, n_ff, LAG * seg, d_main),
                         contract_rest(_load_slabs(act, 0, n_ff, LAG * seg), w2T, 0, n_ff).T], axis=1)
    outs[(n_seg - LAG) * seg:, :] = (res_ffn[...] + y).astype(BF16)
    for b in range(done_blk, n_blk):
        transpose_out(b)
    start(out_late)
    wait(out_early + out_late)


@functools.partial(jax.jit, static_argnames=("A_seg_len",))
def pallas_interleave_layers__memory_aug_recurrent_mem_tr__glu_gated_swiglu__prompt_kernel(
    A_x: jax.Array,
    A_mem0: jax.Array,
    A_Wq: jax.Array,
    A_Wk: jax.Array,
    A_Wv: jax.Array,
    A_Wo: jax.Array,
    A_seg_len: int,
    B_x: jax.Array,
    B_w1: jax.Array,
    B_w3: jax.Array,
    B_w2: jax.Array,
):
    del B_x
    batch, seq, d_model = A_x.shape
    _, n_heads, d_head = A_Wq.shape
    n_mem = A_mem0.shape[1]
    d_ff = B_w1.shape[1]
    seg = int(A_seg_len)
    assert batch == 1 and seq % seg == 0 and seq % TOK_BLOCK == 0
    assert d_head == LANES and d_ff % (4 * LANES) == 0
    assert TOK_BLOCK == (LAG + 1) * seg and seg % 16 == 0 and n_mem % 8 == 0
    assert d_model % 32 == 0 and d_model % LANES != 0 and n_heads % 16 == 0
    rows = 2 * (n_mem + seg)
    n_ff = d_ff // LANES
    n_dm = pl.cdiv(d_model, LANES)

    hbm = pl.BlockSpec(memory_space=pl.ANY)
    outT = pl.pallas_call(
        functools.partial(_kernel, seg=seg, n_mem=n_mem),
        out_shape=jax.ShapeDtypeStruct((d_model, seq), A_x.dtype),
        in_specs=[hbm, pl.BlockSpec(memory_space=pltpu.VMEM)] + [hbm] * 7,
        out_specs=hbm,
        scratch_shapes=[
            pltpu.VMEM((3, d_model * n_heads, d_head), BF16),
            pltpu.VMEM((n_heads, d_model, d_head), BF16),
            pltpu.VMEM((3 * n_ff, d_model, LANES), BF16),
            pltpu.VMEM((3 * n_heads, d_model // 2, d_head), U32),
            pltpu.VMEM((n_heads, d_model // 2, d_head), U32),
            pltpu.VMEM((n_ff, d_model // 2, LANES), U32),
            pltpu.VMEM((n_ff, d_model // 2, LANES), U32),
            pltpu.VMEM((n_ff, d_model // 2, LANES), U32),
            pltpu.VMEM((seq // TOK_BLOCK, d_model, TOK_BLOCK), BF16),
            pltpu.VMEM((seq, d_model), BF16),
            pltpu.VMEM((seq, d_model), BF16),
            pltpu.VMEM((n_dm, rows // 2, LANES), U32),
            pltpu.VMEM((n_dm, LAG * seg // 2, LANES), U32),
            pltpu.VMEM((n_heads, rows // 2, d_head), U32),
            pltpu.VMEM((2 * n_ff, LAG * seg // 2, LANES), U32),
            pltpu.VMEM((LAG * seg, d_model), F32),
            pltpu.VMEM((seg, d_model), F32),
            pltpu.VMEM((2 * (LAG + 1) * seg, d_model), F32),
            pltpu.VMEM((seg, d_model), F32),
            pltpu.VMEM((2 * seg, d_model), F32),
            pltpu.VMEM((rows, rows), F32),
            pltpu.SemaphoreType.DMA((9,)),
            pltpu.SemaphoreType.DMA((6,)),
        ],
        compiler_params=pltpu.CompilerParams(vmem_limit_bytes=100 * 1024 * 1024),
    )(
        A_x[0].T,
        A_mem0[0],
        A_Wq.reshape(d_model * n_heads, d_head),
        A_Wk.reshape(d_model * n_heads, d_head),
        A_Wv.reshape(d_model * n_heads, d_head),
        jnp.transpose(A_Wo, (0, 2, 1)),
        B_w1,
        B_w3,
        B_w2.T,
    )
    return outT.T[None]
```
